```python
import jax
import jax.numpy as jnp

def _softmax(x, axis=-1):
    return jax.nn.softmax(x, axis=axis)

def _gelu(x):
    return jax.nn.gelu(x, approximate=True)

def _silu(x):
    return jax.nn.silu(x)

def _sigmoid(x):
    return jax.nn.sigmoid(x)

def _layernorm(x, axis=-1, eps=1e-05):
    m = jnp.mean(x, axis=axis, keepdims=True)
    v = jnp.var(x, axis=axis, keepdims=True)
    return (x - m) / jnp.sqrt(v + eps)

def _scatter_add(tgt, idx, src, axis=0):
    return tgt.at[idx].add(src)

def _segment_sum(src, seg, n):
    return jax.ops.segment_sum(src, seg, n)

class _Rng:

    def __init__(self, key):
        self._k = key

    def _next(self):
        self._k, sub = jax.random.split(self._k)
        return sub

    def normal(self, shape):
        return jax.random.normal(self._next(), shape, dtype=jnp.bfloat16)

    def randint(self, lo, hi, shape):
        return jax.random.randint(self._next(), shape, lo, hi, dtype=jnp.int32)

    def uniform(self, shape, lo=0.0, hi=1.0):
        return jax.random.uniform(self._next(), shape, jnp.bfloat16, lo, hi)

    def permutation(self, n):
        return jax.random.permutation(self._next(), n)
kernel_name = 'adaLN_cond__compressed_kv_cla__mixer_s_mlp__prompt'

def setup_inputs():
    _rng = _Rng(jax.random.key(int.from_bytes(__import__("os").urandom(4), "little")))
    _w = lambda a: (lambda t: t.astype(jnp.bfloat16) if jnp.issubdtype(t.dtype, jnp.floating) else t)(jnp.asarray(a))

    def _A_setup():
        B, H, Sq, Sk, D, M = (1, 32, 2048, 2048, 128, 640)
        Dc = 4 * D
        return {'x': _w((lambda *s: _rng.normal(s) * 0.05)(B, Sq, M)), 'c_kv': _w((lambda *s: _rng.normal(s) * 0.05)(B, Sk, Dc)), 'w_q': _w((lambda *s: _rng.normal(s) * 0.05)(M, H, D) * M ** (-0.5)), 'w_uk': _w((lambda *s: _rng.normal(s) * 0.05)(Dc, H, D) * Dc ** (-0.5)), 'w_uv': _w((lambda *s: _rng.normal(s) * 0.05)(Dc, H, D) * Dc ** (-0.5)), 'w_o': _w((lambda *s: _rng.normal(s) * 0.05)(H, D, M) * (H * D) ** (-0.5))}
    _A_in = _A_setup()

    def _B_setup():
        B, S, D, F = (1, 2048, 640, 1728)
        return {'x': _w((lambda *s: _rng.normal(s) * 0.05)(B, S, D)), 'w1': _w((lambda *s: _rng.normal(s) * 0.05)(D, D) * D ** (-0.5)), 'w2': _w((lambda *s: _rng.normal(s) * 0.05)(D, D) * D ** (-0.5)), 'w3': _w((lambda *s: _rng.normal(s) * 0.05)(D, F) * D ** (-0.5)), 'w4': _w((lambda *s: _rng.normal(s) * 0.05)(F, D) * F ** (-0.5))}
    _B_in = _B_setup()
    return {'A_x': _A_in['x'], 'A_c_kv': _A_in['c_kv'], 'A_w_q': _A_in['w_q'], 'A_w_uk': _A_in['w_uk'], 'A_w_uv': _A_in['w_uv'], 'A_w_o': _A_in['w_o'], 'B_x': _B_in['x'], 'B_w1': _B_in['w1'], 'B_w2': _B_in['w2'], 'B_w3': _B_in['w3'], 'B_w4': _B_in['w4'], 'c': _w((lambda *s: _rng.normal(s) * 0.05)(1, 640)), 'w_mod': _w((lambda *s: _rng.normal(s) * 0.05)(640, 6 * 640) * 640 ** (-0.5))}

def reference(A_x, A_c_kv, A_w_q, A_w_uk, A_w_uv, A_w_o, B_x, B_w1, B_w2, B_w3, B_w4, c, w_mod):

    def _A_ref(x, c_kv, w_q, w_uk, w_uv, w_o):
        B, Sq, M = (x.shape[0], x.shape[1], x.shape[2])
        Sk = c_kv.shape[1]
        H, D = (w_q.shape[1], w_q.shape[2])
        q = jnp.einsum('bqm,mhd->bhqd', x, w_q)
        k = jnp.einsum('bkc,chd->bhkd', c_kv, w_uk)
        v = jnp.einsum('bkc,chd->bhkd', c_kv, w_uv)
        scores = jnp.einsum('bhqd,bhkd->bhqk', q, k) * D ** (-0.5)
        off = Sk - Sq
        qi = jnp.arange(Sq)[:, None]
        kj = jnp.arange(Sk)[None, :]
        cmask = kj <= qi + off
        scores = jnp.where(cmask[None, None], scores, -1000000000.0)
        p = _softmax(scores, axis=-1)
        ctx = jnp.einsum('bhqk,bhkd->bhqd', p, v)
        return jnp.einsum('bhqd,hdm->bqm', ctx, w_o)

    def _B_ref(x, w1, w2, w3, w4):
        B, S, D = x.shape
        h = _gelu(_layernorm(x, axis=-1) @ w1)
        c = D // 4
        g0 = jnp.pad(h[:, :, 0 * c:1 * c], ((0, 0), (1, 0), (0, 0)))[:, :S, :]
        g1 = jnp.pad(h[:, :, 1 * c:2 * c], ((0, 0), (0, 1), (0, 0)))[:, 1:, :]
        g2 = jnp.pad(h[:, :, 2 * c:3 * c], ((0, 0), (2, 0), (0, 0)))[:, :S, :]
        g3 = jnp.pad(h[:, :, 3 * c:], ((0, 0), (0, 2), (0, 0)))[:, 2:, :]
        hs = jnp.concatenate([g0, g1, g2, g3], axis=-1) @ w2
        x1 = x + hs
        h2 = _gelu(_layernorm(x1, axis=-1) @ w3) @ w4
        return x1 + h2
    x = A_x
    mod = (_silu(c) @ w_mod).reshape(c.shape[0], 6, 1, -1)
    sa, ca, ga, sb, cb, gb = (mod[:, 0].copy(), mod[:, 1].copy(), mod[:, 2].copy(), mod[:, 3].copy(), mod[:, 4].copy(), mod[:, 5].copy())
    h = _layernorm(x, axis=-1) * (1 + ca) + sa
    x = x + ga * _A_ref(h, A_c_kv, A_w_q, A_w_uk, A_w_uv, A_w_o)
    h = _layernorm(x, axis=-1) * (1 + cb) + sb
    x = x + gb * _B_ref(h, B_w1, B_w2, B_w3, B_w4)
    return x
```

```python
import functools
import math
import numpy as np
import jax
import jax.numpy as jnp
from jax import lax
import jax.experimental.pallas as pl
import jax.experimental.pallas.tpu as pltpu

S, M, DC, H, D, F = 2048, 640, 512, 32, 128, 1728
LOG2E = math.log2(math.e)
NEG = -1e9 * LOG2E
BF = jnp.bfloat16
F32 = jnp.float32


def _ln(x):
    m = jnp.mean(x, axis=-1, keepdims=True)
    d = x - m
    v = jnp.mean(d * d, axis=-1, keepdims=True)
    return d * lax.rsqrt(v + 1e-5)


def _gelu(x):
    k0 = math.sqrt(2.0 / math.pi)
    return 0.5 * x * (1.0 + jnp.tanh(k0 * (x + 0.044715 * (x * x * x))))


def _dot(a, b):
    return jnp.dot(a, b, preferred_element_type=F32)


def _dot_nt(a, b):
    return lax.dot_general(a, b, (((1,), (1,)), ((), ())), preferred_element_type=F32)


def make(bq=256, rb=256, vmem_mb=110, attn_mode="full"):
    nq = S // bq
    nrb = S // rb

    def kernel(x_hbm, ckv_hbm, wq_hbm, wuk_hbm, wuv_hbm, wo_hbm, w1_hbm, w2_hbm, w3_hbm, w4_hbm,
               c_hbm, wmod_hbm, out_hbm,
               x_v, ckv_v, wq_v, wuk_v, wuv_v, wo_v, w1_v, w2_v, w3_v, w4_v, c_v, wmod_v,
               h1_s, q_s, k_s, v_s, wq2, wk2, wv2, ctx_s, xa_s, hb_s, t_s, mod_s, ostage, sems, osem):
        srcs = [c_hbm, wmod_hbm, x_hbm, ckv_hbm, wuk_hbm, wuv_hbm, wq_hbm, wo_hbm, w1_hbm, w2_hbm, w3_hbm, w4_hbm]
        dsts = [c_v, wmod_v, x_v, ckv_v, wuk_v, wuv_v, wq_v, wo_v, w1_v, w2_v, w3_v, w4_v]
        cps = [pltpu.make_async_copy(s, d, sems.at[i]) for i, (s, d) in enumerate(zip(srcs, dsts))]
        for cp in cps:
            cp.start()
        cps[0].wait(); cps[1].wait()
        cc = c_v[...].astype(F32)
        sc = (cc * jax.nn.sigmoid(cc)).astype(BF)
        mod_s[...] = _dot(sc, wmod_v[...])
        cps[2].wait()
        sa = mod_s[:, 0:M]
        ca = mod_s[:, M:2 * M]

        def ln1(i, _):
            r = pl.multiple_of(i * rb, rb)
            xx = x_v[pl.ds(r, rb), :].astype(F32)
            h1_s[pl.ds(r, rb), :] = (_ln(xx) * (1.0 + ca) + sa).astype(BF)
            return 0
        lax.fori_loop(0, nrb, ln1, 0)
        cps[3].wait(); cps[4].wait(); cps[5].wait(); cps[6].wait()

        wq32 = wq_v.bitcast(jnp.uint32)
        wk32 = wuk_v.bitcast(jnp.uint32)
        wv32 = wuv_v.bitcast(jnp.uint32)

        def pair_w(ref32, rows, p):
            b = ref32[pl.ds(p, rows, stride=H // 2), :]
            lo = pltpu.bitcast(b << 16, F32).astype(BF)
            hi = pltpu.bitcast(b & jnp.uint32(0xFFFF0000), F32).astype(BF)
            return lo, hi

        for (r32, rows, dst) in ((wk32, DC, wk2), (wv32, DC, wv2), (wq32, M, wq2)):
            for p in range(H // 2):
                lo, hi = pair_w(r32, rows, p)
                dst[p, :, 0:D] = lo
                dst[p, :, D:2 * D] = hi

        row_i = lax.broadcasted_iota(jnp.int32, (bq, bq), 0)
        col_i = lax.broadcasted_iota(jnp.int32, (bq, bq), 1)

        def attn(j, hd):
            for i in range(nq):
                q = q_s[i * bq:(i + 1) * bq, j * D:(j + 1) * D]
                kl = (i + 1) * bq
                s = _dot_nt(q, k_s[0:kl, j * D:(j + 1) * D])
                sd = jnp.where(col_i <= row_i, s[:, kl - bq:], NEG)
                if i > 0:
                    s = jnp.concatenate([s[:, :kl - bq], sd], axis=1)
                else:
                    s = sd
                m = jnp.max(s, axis=1, keepdims=True)
                p = jnp.exp2(s - m)
                l = jnp.sum(p, axis=1, keepdims=True)
                o = _dot(p.astype(BF), v_s[0:kl, j * D:(j + 1) * D]) / l
                ctx_s[hd, i * bq:(i + 1) * bq, :] = o.astype(BF)

        def pair_body(p, _):
            ckv = ckv_v[...]
            h1 = h1_s[...]
            k_s[...] = _dot(ckv, wk2[p]).astype(BF)
            v_s[...] = _dot(ckv, wv2[p]).astype(BF)
            q_s[...] = (_dot(h1, wq2[p]) * (D ** -0.5 * LOG2E)).astype(BF)
            for j in range(2):
                attn(j, 2 * p + j)
            return 0
        lax.fori_loop(0, H // 2, pair_body, 0)

        cps[7].wait(); cps[8].wait()
        ga = mod_s[:, 2 * M:3 * M]
        sb = mod_s[:, 3 * M:4 * M]
        cb = mod_s[:, 4 * M:5 * M]
        gb = mod_s[:, 5 * M:6 * M]
        zpad = jnp.zeros((8, M), F32)
        t_s[0:8, :] = zpad
        t_s[S + 8:S + 16, :] = zpad

        def mlp1(i, _):
            r = pl.multiple_of(i * rb, rb)
            acc = jnp.zeros((rb, M), F32)
            for hd in range(H):
                acc += _dot(ctx_s[hd, pl.ds(r, rb), :], wo_v[hd * D:(hd + 1) * D, :])
            xa = x_v[pl.ds(r, rb), :].astype(F32) + ga * acc
            xa_s[pl.ds(r, rb), :] = xa
            hb = _ln(xa) * (1.0 + cb) + sb
            hb_s[pl.ds(r, rb), :] = hb
            t = _gelu(_dot(_ln(hb).astype(BF), w1_v[...]))
            t_s[pl.ds(pl.multiple_of(r + 8, 8), rb), :] = t
            return 0
        lax.fori_loop(0, nrb, mlp1, 0)

        cps[9].wait(); cps[10].wait(); cps[11].wait()
        lane = lax.broadcasted_iota(jnp.int32, (rb, 128), 1)
        G = M // 4
        offs = (-1, 1, -2, 2)

        def mlp2(i, _):
            r = pl.multiple_of(i * rb, rb)
            cols = []
            for ct in range(M // 128):
                g_lo = (ct * 128) // G
                g_hi = (ct * 128 + 127) // G
                w = t_s[pl.ds(r, rb + 16), ct * 128:(ct + 1) * 128]
                a = w[8 + offs[g_lo]:8 + offs[g_lo] + rb]
                if g_hi != g_lo:
                    b = w[8 + offs[g_hi]:8 + offs[g_hi] + rb]
                    a = jnp.where(lane < (g_hi * G - ct * 128), a, b)
                cols.append(a)
            g = jnp.concatenate(cols, axis=1).astype(BF)
            y1 = hb_s[pl.ds(r, rb), :] + _dot(g, w2_v[...])
            u = _gelu(_dot_nt(_ln(y1).astype(BF), w3_v[...])).astype(BF)
            y2 = y1 + _dot(u, w4_v[...])
            o = xa_s[pl.ds(r, rb), :] + gb * y2
            slot = i % 2

            @pl.when(i >= 2)
            def _():
                pltpu.make_async_copy(ostage.at[slot], out_hbm.at[pl.ds(r, rb), :], osem.at[slot]).wait()
            ostage[slot] = o.astype(BF)
            pltpu.make_async_copy(ostage.at[slot], out_hbm.at[pl.ds(r, rb), :], osem.at[slot]).start()
            return 0
        lax.fori_loop(0, nrb, mlp2, 0)
        for slot in range(2):
            pltpu.make_async_copy(ostage.at[slot], out_hbm.at[pl.ds(0, rb), :], osem.at[slot]).wait()

    scratch = [
        pltpu.VMEM((S, M), BF), pltpu.VMEM((S, DC), BF),
        pltpu.VMEM((M * H, D), BF), pltpu.VMEM((DC * H, D), BF), pltpu.VMEM((DC * H, D), BF),
        pltpu.VMEM((H * D, M), BF), pltpu.VMEM((M, M), BF), pltpu.VMEM((M, M), BF),
        pltpu.VMEM((F, M), BF), pltpu.VMEM((F, M), BF), pltpu.VMEM((1, M), BF), pltpu.VMEM((M, 6 * M), BF),
        pltpu.VMEM((S, M), BF),
        pltpu.VMEM((S, 2 * D), BF), pltpu.VMEM((S, 2 * D), BF), pltpu.VMEM((S, 2 * D), BF),
        pltpu.VMEM((H // 2, M, 2 * D), BF), pltpu.VMEM((H // 2, DC, 2 * D), BF), pltpu.VMEM((H // 2, DC, 2 * D), BF),
        pltpu.VMEM((H, S, D), BF),
        pltpu.VMEM((S, M), F32), pltpu.VMEM((S, M), F32), pltpu.VMEM((S + 16, M), F32),
        pltpu.VMEM((1, 6 * M), F32), pltpu.VMEM((2, rb, M), BF),
        pltpu.SemaphoreType.DMA((12,)), pltpu.SemaphoreType.DMA((2,)),
    ]

    @jax.jit
    def fn(A_x, A_c_kv, A_w_q, A_w_uk, A_w_uv, A_w_o, B_x, B_w1, B_w2, B_w3, B_w4, c, w_mod):
        any_spec = pl.BlockSpec(memory_space=pltpu.HBM)
        out = pl.pallas_call(
            kernel,
            out_shape=jax.ShapeDtypeStruct((S, M), BF),
            in_specs=[any_spec] * 12,
            out_specs=any_spec,
            scratch_shapes=scratch,
            compiler_params=pltpu.CompilerParams(vmem_limit_bytes=vmem_mb * 1024 * 1024),
        )(A_x.reshape(S, M), A_c_kv.reshape(S, DC), A_w_q.reshape(M * H, D), A_w_uk.reshape(DC * H, D),
          A_w_uv.reshape(DC * H, D), A_w_o.reshape(H * D, M), B_w1, B_w2, B_w3.T, B_w4, c, w_mod)
        return out.reshape(1, S, M)
    return fn


_kernel = make()


def pallas_adaLN_cond__compressed_kv_cla__mixer_s_mlp__prompt_kernel(
    A_x, A_c_kv, A_w_q, A_w_uk, A_w_uv, A_w_o, B_x, B_w1, B_w2, B_w3, B_w4, c, w_mod
):
    return _kernel(A_x, A_c_kv, A_w_q, A_w_uk, A_w_uv, A_w_o, B_x, B_w1, B_w2, B_w3, B_w4, c, w_mod)
```

```python
import functools
import math
import numpy as np
import jax
import jax.numpy as jnp
from jax import lax
import jax.experimental.pallas as pl
import jax.experimental.pallas.tpu as pltpu

S, M, DC, H, D, F = 2048, 640, 512, 32, 128, 1728
LOG2E = math.log2(math.e)
NEG = -1e9 * LOG2E
QSCALE = D ** -0.5 * LOG2E
BF = jnp.bfloat16
F32 = jnp.float32
U32 = jnp.uint32
GH = 16


def _ln(x):
    m = jnp.mean(x, axis=-1, keepdims=True)
    d = x - m
    v = jnp.mean(d * d, axis=-1, keepdims=True)
    return d * lax.rsqrt(v + 1e-5)


def _gelu(x):
    k0 = math.sqrt(2.0 / math.pi)
    return 0.5 * x * (1.0 + jnp.tanh(k0 * (x + 0.044715 * (x * x * x))))


def _dot(a, b):
    return jnp.dot(a, b, preferred_element_type=F32)


def _dot_nt(a, b):
    return lax.dot_general(a, b, (((1,), (1,)), ((), ())), preferred_element_type=F32)


def _transpose8(vs):
    sl = lax.broadcasted_iota(jnp.int32, vs[0].shape, 1)
    for d in (4, 2, 1):
        msk = (sl & d) == 0
        nv = list(vs)
        for i in range(8):
            if i & d:
                continue
            a, b = vs[i], vs[i + d]
            nv[i] = jnp.where(msk, a, pltpu.roll(b, d, 1))
            nv[i + d] = jnp.where(msk, pltpu.roll(a, 8 - d, 1), b)
        vs = nv
    return vs


def _relayout(raw, g, m0, nrows, dst, gd, sub=16):
    for c in range(nrows // sub):
        r0 = m0 + c * sub
        if not isinstance(r0, int):
            r0 = pl.multiple_of(r0, 16)
        x = raw[g, pl.ds(r0, sub), :, :]
        b = pltpu.bitcast(x, U32).reshape(sub // 8, 8, 8, 128)
        vs = _transpose8([b[:, i] for i in range(8)])
        for j in range(8):
            v = vs[j].reshape(sub, 128)
            dst[gd * GH + 2 * j, pl.ds(r0, sub), :] = pltpu.bitcast(v << 16, F32).astype(BF)
            dst[gd * GH + 2 * j + 1, pl.ds(r0, sub), :] = pltpu.bitcast(v & jnp.uint32(0xFFFF0000), F32).astype(BF)


def make(rb=512, vmem_mb=110, order="mount", pc=128, lnb=256, fillpos="after", lead=0, peel=False, approx=False, rb2=512, flags=None):
    bq = 128
    nrb = S // rb
    ns = S // bq

    def kernel(x_hbm, ckv_hbm, wq_hbm, wk_hbm, wv_hbm, wo_hbm, w1_hbm, w2_hbm, w3_hbm, w4_hbm,
               c_hbm, wmod_hbm, out_hbm,
               x_v, ckv_v, wq_v, wk_v, wv_v, wo_v, w1_v, w2_v, w3_v, w4_v, c_v, wmod_v,
               h1_s, wq2, wk2, wv2, ctx_s, xa_s, hb_s, t_s, mod_s, ostage,
               sems, osem):
        def cp(i, src, dst):
            return pltpu.make_async_copy(src, dst, sems.at[i])

        c_c = cp(0, c_hbm, c_v)
        c_wm0 = cp(1, wmod_hbm.at[:, 0:2 * M], wmod_v.at[:, 0:2 * M])
        c_x = cp(2, x_hbm, x_v)
        c_ckv = cp(3, ckv_hbm, ckv_v)
        c_wk = [cp(4 + g, wk_hbm.at[:, g * GH:(g + 1) * GH, :], wk_v.at[g]) for g in range(2)]
        c_wv = [cp(6 + g, wv_hbm.at[:, g * GH:(g + 1) * GH, :], wv_v.at[g]) for g in range(2)]
        c_wq = [cp(8 + g, wq_hbm.at[:, g * GH:(g + 1) * GH, :], wq_v.at[g]) for g in range(2)]
        c_wm1 = cp(10, wmod_hbm.at[:, 2 * M:6 * M], wmod_v.at[:, 2 * M:6 * M])
        c_wo = cp(11, wo_hbm, wo_v)
        c_w1 = cp(12, w1_hbm, w1_v)
        c_w2 = cp(13, w2_hbm, w2_v)
        c_w3 = cp(14, w3_hbm, w3_v)
        c_w4 = cp(15, w4_hbm, w4_v)

        for q in (c_c, c_wm0, c_wk[0], c_ckv, c_x, c_wv[0], c_wq[0]):
            q.start()
        c_c.wait()
        c_wm0.wait()
        cc = c_v[...].astype(F32)
        sc = (cc * jax.nn.sigmoid(cc)).astype(BF)
        mod_s[:, 0:2 * M] = _dot(sc, wmod_v[:, 0:2 * M])
        c_wk[0].wait()
        _relayout(wk_v, 0, 0, DC, wk2, 0)
        c_x.wait()
        sa = mod_s[:, 0:M]
        ca = mod_s[:, M:2 * M]

        def ln1(i, _):
            r = pl.multiple_of(i * lnb, lnb)
            xx = x_v[pl.ds(r, lnb), :].astype(F32)
            h1_s[pl.ds(r, lnb), :] = (_ln(xx) * (1.0 + ca) + sa).astype(BF)
            return 0
        lax.fori_loop(0, S // lnb, ln1, 0)
        c_wv[0].wait()
        _relayout(wv_v, 0, 0, DC, wv2, 0)
        c_wq[0].wait()
        for q in (c_wk[1], c_wv[1], c_wq[1]):
            q.start()
        _relayout(wq_v, 0, 0, M, wq2, 0)
        c_ckv.wait()

        def proj_pieces(h, qd, kd, vd):
            pcs = []
            for r in range(S // pc):
                rs = slice(r * pc, (r + 1) * pc)
                pcs.append(lambda rs=rs: kd.__setitem__((rs, slice(None)), _dot(ckv_v[rs, :], wk2[h]).astype(BF)))
                pcs.append(lambda rs=rs: vd.__setitem__((rs, slice(None)), _dot(ckv_v[rs, :], wv2[h]).astype(BF)))
                pcs.append(lambda rs=rs: qd.__setitem__((rs, slice(None)), (_dot(h1_s[rs, :], wq2[h]) * QSCALE).astype(BF)))
            return pcs

        row_i = lax.broadcasted_iota(jnp.int32, (128, 128), 0)
        col_i = lax.broadcasted_iota(jnp.int32, (128, 128), 1)
        tri = col_i <= row_i

        qa, ka, va, qb, kb, vb = [ctx_s.at[H + i] for i in range(6)]

        def qk(i, qs, ks):
            q0 = i * bq
            s = _dot_nt(qs[q0:q0 + bq, :], ks[0:q0 + bq, :])
            sd = jnp.where(tri, s[:, q0:], NEG)
            return jnp.concatenate([s[:, :q0], sd], axis=1) if i > 0 else sd

        def sm(s):
            m = jnp.max(s, axis=1, keepdims=True)
            p = jnp.exp2(s - m)
            l = jnp.sum(p, axis=1, keepdims=True)
            return p.astype(BF), l

        def pv(i, hd, pl_, vs):
            q0 = i * bq
            p, l = pl_
            o = _dot(p, vs[0:q0 + bq, :])
            if approx:
                o = o * pl.reciprocal(l, approx=True)
            else:
                o = o / l
            ctx_s[hd, q0:q0 + bq, :] = o.astype(BF)

        def head_order():
            idx = list(range(ns))
            if order == "desc":
                return idx[::-1]
            if order == "asc":
                return idx
            return idx[0::2] + idx[1::2][::-1]

        def alloc(nf, w):
            tot = sum(w)
            acc = 0.0
            out = []
            done = 0
            for x in w:
                acc += x
                k = int(round(nf * acc / tot)) - done
                out.append(k)
                done += k
            return out

        def unified(hA, hB, fA, fB):
            ho = head_order()
            tasks = [(hA, i, qa, ka, va) for i in ho] + [(hB, i, qb, kb, vb) for i in ho]
            ws = [0.0 if n >= ns - lead else 1.0 for n in range(ns)]
            alA = alloc(len(fA), ws)
            alB = alloc(len(fB), ws)
            nt = len(tasks)
            nxt = qk(tasks[0][1], tasks[0][2], tasks[0][3])
            prevp = None
            for n, (hd, i, q_, k_, v_) in enumerate(tasks):
                ss = nxt
                fl, al = (fA, alA) if n < ns else (fB, alB)

                def dofill():
                    for _ in range(al[n % ns]):
                        fl.pop(0)()
                if fillpos == "first":
                    dofill()
                if n + 1 < nt:
                    t = tasks[n + 1]
                    nxt = qk(t[1], t[2], t[3])
                if prevp is not None:
                    t = tasks[n - 1]
                    pv(t[1], t[0], prevp, t[4])
                if fillpos == "mid2":
                    dofill()
                prevp = sm(ss)
                if fillpos == "after":
                    dofill()
            t = tasks[-1]
            pv(t[1], t[0], prevp, t[4])
            assert not fA and not fB

        for f in proj_pieces(0, qa, ka, va):
            f()

        def pair_body(p, _):
            g = p // 8
            gn = jnp.minimum(g + 1, 1)

            @pl.when(p == 0)
            def _():
                c_wk[1].wait()
                c_wv[1].wait()
                c_wq[1].wait()
                for q in (c_wm1, c_wo, c_w1, c_w2, c_w3, c_w4):
                    q.start()
            ch = p % 8
            rl = [
                lambda: _relayout(wk_v, gn, ch * (DC // 8), DC // 8, wk2, (g + 1) % 2),
                lambda: _relayout(wv_v, gn, ch * (DC // 8), DC // 8, wv2, (g + 1) % 2),
                lambda: _relayout(wq_v, gn, ch * (M // 8), M // 8, wq2, (g + 1) % 2),
            ]
            fA = proj_pieces(2 * p + 1, qb, kb, vb)
            n = len(fA)
            fA = fA[:n // 4] + rl[0:1] + fA[n // 4:n // 2] + rl[1:2] + fA[n // 2:3 * n // 4] + rl[2:3] + fA[3 * n // 4:]
            hn = jnp.minimum(2 * p + 2, H - 1)
            unified(2 * p, 2 * p + 1, fA, proj_pieces(hn, qa, ka, va))
            return 0
        lax.fori_loop(0, H // 2, pair_body, 0)

        c_wm1.wait()
        mod_s[:, 2 * M:6 * M] = _dot(sc, wmod_v[:, 2 * M:6 * M])
        c_wo.wait()
        c_w1.wait()
        ga = mod_s[:, 2 * M:3 * M]
        sb = mod_s[:, 3 * M:4 * M]
        cb = mod_s[:, 4 * M:5 * M]
        gb = mod_s[:, 5 * M:6 * M]
        zpad = jnp.zeros((8, M), F32)
        t_s[0:8, :] = zpad
        t_s[S + 8:S + 16, :] = zpad

        def mlp1(i, _):
            r = pl.multiple_of(i * rb, rb)
            acc = jnp.zeros((rb, M), F32)
            for hd in range(H):
                acc += _dot(ctx_s[hd, pl.ds(r, rb), :], wo_v[hd * D:(hd + 1) * D, :])
            xa = x_v[pl.ds(r, rb), :].astype(F32) + ga * acc
            xa_s[pl.ds(r, rb), :] = xa
            hb = _ln(xa) * (1.0 + cb) + sb
            hb_s[pl.ds(r, rb), :] = hb
            t = _gelu(_dot(_ln(hb).astype(BF), w1_v[...]))
            t_s[pl.ds(pl.multiple_of(r + 8, 8), rb), :] = t
            return 0
        lax.fori_loop(0, nrb, mlp1, 0)

        c_w2.wait()
        c_w3.wait()
        c_w4.wait()
        lane = lax.broadcasted_iota(jnp.int32, (rb2, 128), 1)
        G = M // 4
        offs = (-1, 1, -2, 2)

        def mlp2(i, _):
            r = pl.multiple_of(i * rb2, rb2)
            cols = []
            for ct in range(M // 128):
                g_lo = (ct * 128) // G
                g_hi = (ct * 128 + 127) // G
                w = t_s[pl.ds(r, rb2 + 16), ct * 128:(ct + 1) * 128]
                a = w[8 + offs[g_lo]:8 + offs[g_lo] + rb2]
                if g_hi != g_lo:
                    b = w[8 + offs[g_hi]:8 + offs[g_hi] + rb2]
                    a = jnp.where(lane < (g_hi * G - ct * 128), a, b)
                cols.append(a)
            g = jnp.concatenate(cols, axis=1).astype(BF)
            y1 = hb_s[pl.ds(r, rb2), :] + _dot(g, w2_v[...])
            u = _gelu(_dot_nt(_ln(y1).astype(BF), w3_v[...])).astype(BF)
            y2 = y1 + _dot(u, w4_v[...])
            o = xa_s[pl.ds(r, rb2), :] + gb * y2
            slot = i % 2

            @pl.when(i >= 2)
            def _():
                pltpu.make_async_copy(ostage.at[slot], out_hbm.at[pl.ds(r, rb2), :], osem.at[slot]).wait()
            ostage[slot] = o.astype(BF)
            pltpu.make_async_copy(ostage.at[slot], out_hbm.at[pl.ds(r, rb2), :], osem.at[slot]).start()
            return 0
        lax.fori_loop(0, S // rb2, mlp2, 0)
        for slot in range(2):
            pltpu.make_async_copy(ostage.at[slot], out_hbm.at[pl.ds(0, rb2), :], osem.at[slot]).wait()

    scratch = [
        pltpu.VMEM((S, M), BF), pltpu.VMEM((S, DC), BF),
        pltpu.VMEM((2, M, GH, D), BF), pltpu.VMEM((2, DC, GH, D), BF), pltpu.VMEM((2, DC, GH, D), BF),
        pltpu.VMEM((H * D, M), BF), pltpu.VMEM((M, M), BF), pltpu.VMEM((M, M), BF),
        pltpu.VMEM((F, M), BF), pltpu.VMEM((F, M), BF), pltpu.VMEM((1, M), BF), pltpu.VMEM((M, 6 * M), BF),
        pltpu.VMEM((S, M), BF),
        pltpu.VMEM((H, M, D), BF), pltpu.VMEM((H, DC, D), BF), pltpu.VMEM((H, DC, D), BF),
        pltpu.VMEM((H + 6, S, D), BF),
        pltpu.VMEM((S, M), F32), pltpu.VMEM((S, M), F32), pltpu.VMEM((S + 16, M), F32),
        pltpu.VMEM((1, 6 * M), F32), pltpu.VMEM((2, rb2, M), BF),
        pltpu.SemaphoreType.DMA((16,)), pltpu.SemaphoreType.DMA((2,)),
    ]

    @jax.jit
    def fn(A_x, A_c_kv, A_w_q, A_w_uk, A_w_uv, A_w_o, B_x, B_w1, B_w2, B_w3, B_w4, c, w_mod):
        hbm = pl.BlockSpec(memory_space=pltpu.HBM)
        out = pl.pallas_call(
            kernel,
            out_shape=jax.ShapeDtypeStruct((S, M), BF),
            in_specs=[hbm] * 12,
            out_specs=hbm,
            scratch_shapes=scratch,
            compiler_params=pltpu.CompilerParams(vmem_limit_bytes=vmem_mb * 1024 * 1024, flags=flags),
        )(A_x.reshape(S, M), A_c_kv.reshape(S, DC), A_w_q, A_w_uk, A_w_uv, A_w_o.reshape(H * D, M),
          B_w1, B_w2, B_w3.T, B_w4, c, w_mod)
        return out.reshape(1, S, M)
    return fn


_kernel = make()


def pallas_adaLN_cond__compressed_kv_cla__mixer_s_mlp__prompt_kernel(
    A_x, A_c_kv, A_w_q, A_w_uk, A_w_uv, A_w_o, B_x, B_w1, B_w2, B_w3, B_w4, c, w_mod
):
    return _kernel(A_x, A_c_kv, A_w_q, A_w_uk, A_w_uv, A_w_o, B_x, B_w1, B_w2, B_w3, B_w4, c, w_mod)
```

```python
import math
import jax
import jax.numpy as jnp
from jax import lax
import jax.experimental.pallas as pl
import jax.experimental.pallas.tpu as pltpu

S, M, DC, H, D, F = 2048, 640, 512, 32, 128, 1728
LOG2E = math.log2(math.e)
NEG = -1e9 * LOG2E
QSCALE = D ** -0.5 * LOG2E
BF = jnp.bfloat16
F32 = jnp.float32
U32 = jnp.uint32
GH = 16
BQ = 128


def _ln(x):
    m = jnp.mean(x, axis=-1, keepdims=True)
    d = x - m
    v = jnp.mean(d * d, axis=-1, keepdims=True)
    return d * lax.rsqrt(v + 1e-5)


def _gelu(x):
    k0 = math.sqrt(2.0 / math.pi)
    return 0.5 * x * (1.0 + jnp.tanh(k0 * (x + 0.044715 * (x * x * x))))


def _dot(a, b):
    return jnp.dot(a, b, preferred_element_type=F32)


def _dot_nt(a, b):
    return lax.dot_general(a, b, (((1,), (1,)), ((), ())), preferred_element_type=F32)


def _al(r, n):
    return r if isinstance(r, int) else pl.multiple_of(r, n)


def _transpose8(vs):
    sl = lax.broadcasted_iota(jnp.int32, vs[0].shape, 1)
    for d in (4, 2, 1):
        msk = (sl & d) == 0
        nv = list(vs)
        for i in range(8):
            if i & d:
                continue
            a, b = vs[i], vs[i + d]
            nv[i] = jnp.where(msk, a, pltpu.roll(b, d, 1))
            nv[i + d] = jnp.where(msk, pltpu.roll(a, 8 - d, 1), b)
        vs = nv
    return vs


def _relayout16(raw, g, r0, dst):
    x = raw[g, pl.ds(_al(r0, 16), 16), :, :]
    b = pltpu.bitcast(x, U32).reshape(2, 8, 8, 128)
    vs = _transpose8([b[:, i] for i in range(8)])
    for j in range(8):
        v = vs[j].reshape(16, 128)
        dst[g * GH + 2 * j, pl.ds(_al(r0, 16), 16), :] = pltpu.bitcast(v << 16, F32).astype(BF)
        dst[g * GH + 2 * j + 1, pl.ds(_al(r0, 16), 16), :] = pltpu.bitcast(v & jnp.uint32(0xFFFF0000), F32).astype(BF)


def _spread(a, b):
    out = []
    nb = 0
    for i, x in enumerate(a):
        out.append(x)
        while nb < len(b) and (nb + 1) * len(a) <= (i + 1) * (len(b) + 0):
            out.append(b[nb])
            nb += 1
    out.extend(b[nb:])
    return out


def make(rb=512, sub=128, vmem_mb=110, order="mount", pc=128, fillpos="after", scopes=False, nx=4, pro=0, rlw="AB", dma_at=1, perm=("ckv_v", "h1_s", "wq2", "wk2", "wv2", "ctx_s"), seq="PFQ", div="newton", peel=True, nck=4, opaque=True, firstrl=True, dynrl=False, earlywait=False, lastseq="QP", lastorder="mount", opq_last=False, flags=None):
    ns = S // BQ
    import contextlib
    scope = jax.named_scope if scopes else (lambda name: contextlib.nullcontext())

    names = ["x_v", "ckv_v", "wq_v", "wk_v", "wv_v", "wo_v", "w1_v", "w2_v", "w3_v", "w4_v", "c_v", "wmod_v",
             "h1_s", "wq2", "wk2", "wv2", "ctx_s", "xa_s", "hb_s", "t_s", "mod_s", "ostage"]
    if perm is not None:
        names = list(perm) + [n for n in names if n not in perm]

    def kernel(x_hbm, ckv_hbm, wq_hbm, wk_hbm, wv_hbm, wo_hbm, w1_hbm, w2_hbm, w3_hbm, w4_hbm,
               c_hbm, wmod_hbm, out_hbm, *scr):
        R = dict(zip(names, scr[:len(names)]))
        sems, xsem, osem, csem, pidx = scr[len(names):]
        x_v, ckv_v, wq_v, wk_v, wv_v, wo_v, w1_v, w2_v, w3_v, w4_v, c_v, wmod_v = [R[n] for n in
            ("x_v", "ckv_v", "wq_v", "wk_v", "wv_v", "wo_v", "w1_v", "w2_v", "w3_v", "w4_v", "c_v", "wmod_v")]
        h1_s, wq2, wk2, wv2, ctx_s, xa_s, hb_s, t_s, mod_s, ostage = [R[n] for n in
            ("h1_s", "wq2", "wk2", "wv2", "ctx_s", "xa_s", "hb_s", "t_s", "mod_s", "ostage")]

        def cp(i, src, dst):
            return pltpu.make_async_copy(src, dst, sems.at[i])

        xr = S // nx
        c_c = cp(0, c_hbm, c_v)
        c_wm0 = cp(1, wmod_hbm.at[:, 0:2 * M], wmod_v.at[:, 0:2 * M])
        c_x = [pltpu.make_async_copy(x_hbm.at[i * xr:(i + 1) * xr, :], x_v.at[i * xr:(i + 1) * xr, :], xsem.at[i])
               for i in range(nx)]
        c_ckv = cp(3, ckv_hbm, ckv_v)
        c_wk = [cp(4 + g, wk_hbm.at[:, g * GH:(g + 1) * GH, :], wk_v.at[g]) for g in range(2)]
        c_wv = [cp(6 + g, wv_hbm.at[:, g * GH:(g + 1) * GH, :], wv_v.at[g]) for g in range(2)]
        c_wq = [cp(8 + g, wq_hbm.at[:, g * GH:(g + 1) * GH, :], wq_v.at[g]) for g in range(2)]
        c_wm1 = cp(10, wmod_hbm.at[:, 2 * M:6 * M], wmod_v.at[:, 2 * M:6 * M])
        c_wo = cp(11, wo_hbm, wo_v)
        c_w1 = cp(12, w1_hbm, w1_v)
        c_w2 = cp(13, w2_hbm, w2_v)
        c_w3 = cp(14, w3_hbm, w3_v)
        c_w4 = cp(15, w4_hbm, w4_v)

        qa, ka, va, qb, kb, vb = [ctx_s.at[H + i] for i in range(6)]

        def k_piece(h, kd, r0, n):
            kd[r0:r0 + n, :] = _dot(ckv_v[r0:r0 + n, :], wk2[h]).astype(BF)

        def v_piece(h, vd, r0, n):
            vd[r0:r0 + n, :] = _dot(ckv_v[r0:r0 + n, :], wv2[h]).astype(BF)

        def q_piece(h, qd, r0, n):
            qd[r0:r0 + n, :] = (_dot(h1_s[r0:r0 + n, :], wq2[h]) * QSCALE).astype(BF)

        def proj_pieces(h, qd, kd, vd):
            pcs = []
            for r in range(S // pc):
                pcs.append(lambda r=r: k_piece(h, kd, r * pc, pc))
                pcs.append(lambda r=r: v_piece(h, vd, r * pc, pc))
                pcs.append(lambda r=r: q_piece(h, qd, r * pc, pc))
            return pcs

        cr = S // nck
        c_ck = [pltpu.make_async_copy(ckv_hbm.at[i * cr:(i + 1) * cr, :], ckv_v.at[i * cr:(i + 1) * cr, :], csem.at[i])
                for i in range(nck)]
        with scope("p_mod_ln"):
            for q in [c_c, c_wm0] + c_x + ([c_wq[0]] if pro == 0 else []):
                q.start()
            c_c.wait()
            c_wm0.wait()
            (c_wk[0] if pro == 0 else c_wq[0]).start()
            cc = c_v[...].astype(F32)
            sc = (cc * jax.nn.sigmoid(cc)).astype(BF)
            mod_s[:, 0:2 * M] = _dot(sc, wmod_v[:, 0:2 * M])
            sa = mod_s[:, 0:M]
            ca = mod_s[:, M:2 * M]
            for i in range(nx):
                c_x[i].wait()
                if pro == 0 and i == 0:
                    c_wv[0].start()
                if pro == 1 and i == 1:
                    c_wk[0].start()
                if pro == 1 and i == 3:
                    c_wv[0].start()
                for r in range(i * xr, (i + 1) * xr, 256):
                    xx = x_v[r:r + 256, :].astype(F32)
                    h1_s[r:r + 256, :] = (_ln(xx) * (1.0 + ca) + sa).astype(BF)
        with scope("p_q"):
            c_wq[0].wait()
            for q in c_ck:
                q.start()
            for r in range(M // 16):
                _relayout16(wq_v, 0, r * 16, wq2)
            for r in range(S // 512):
                q_piece(0, qa, r * 512, 512)
        with scope("p_kv"):
            c_wk[0].wait()
            for r in range(DC // 16):
                _relayout16(wk_v, 0, r * 16, wk2)
            c_wv[0].wait()
            for q in (c_wk[1], c_wv[1], c_wq[1]):
                q.start()
            for r in range(DC // 16):
                _relayout16(wv_v, 0, r * 16, wv2)
            for i in range(nck):
                c_ck[i].wait()
                k_piece(0, ka, i * cr, cr)
                v_piece(0, va, i * cr, cr)

        row_i = lax.broadcasted_iota(jnp.int32, (BQ, BQ), 0)
        col_i = lax.broadcasted_iota(jnp.int32, (BQ, BQ), 1)
        tri = col_i <= row_i

        def qk(i, qs, ks):
            q0 = i * BQ
            s = _dot_nt(qs[q0:q0 + BQ, :], ks[0:q0 + BQ, :])
            sd = jnp.where(tri, s[:, q0:], NEG)
            return jnp.concatenate([s[:, :q0], sd], axis=1) if i > 0 else sd

        def sm(s):
            m = jnp.max(s, axis=1, keepdims=True)
            p = jnp.exp2(s - m)
            l = jnp.sum(p, axis=1, keepdims=True)
            return p.astype(BF), l

        def pv(i, hd, pl_, vs):
            q0 = i * BQ
            p, l = pl_
            o = _dot(p, vs[0:q0 + BQ, :])
            if div == "div":
                o = o / l
            else:
                o = o * (1.0 / l)
            ctx_s[hd, q0:q0 + BQ, :] = o.astype(BF)

        def head_order():
            idx = list(range(ns))
            if order == "desc":
                return idx[::-1]
            if order == "asc":
                return idx
            return idx[0::2] + idx[1::2][::-1]

        def alloc(nf):
            return [(nf * (n + 1)) // ns - (nf * n) // ns for n in range(ns)]

        def unified(hA, hB, fA, fB, seqB=None, orderB=None):
            ho = head_order()
            hoB = ho if orderB is None else orderB
            tasks = [(hA, i, qa, ka, va) for i in ho] + [(hB, i, qb, kb, vb) for i in hoB]
            alA, alB = alloc(len(fA)), alloc(len(fB))
            nt = len(tasks)
            sv = {0: qk(tasks[0][1], tasks[0][2], tasks[0][3])}
            pvv = {}
            for n in range(nt + 1):
                fl, al = (fA, alA) if n < ns else (fB, alB)
                for ch in (seqB if (seqB and n >= ns) else seq):
                    if ch == "Q" and n + 1 < nt:
                        t = tasks[n + 1]
                        sv[n + 1] = qk(t[1], t[2], t[3])
                    elif ch == "P" and 0 <= n - 1 < nt:
                        t = tasks[n - 1]
                        pv(t[1], t[0], pvv.pop(n - 1), t[4])
                    elif ch == "F" and n < nt:
                        for _ in range(al[n % ns]):
                            fl.pop(0)()
                if n < nt:
                    pvv[n] = sm(sv.pop(n))
            assert not fA and not fB

        def start_mlp_dmas():
            for q in (c_wm1, c_wo, c_w1, c_w2, c_w3, c_w4):
                q.start()

        def wait_g1():
            c_wk[1].wait()
            c_wv[1].wait()
            c_wq[1].wait()

        def rl_pieces(g, rk, rq, uk, uq):
            rl = [lambda u=u: _relayout16(wk_v, g, rk + u * 16, wk2) for u in range(uk)]
            rl += [lambda u=u: _relayout16(wv_v, g, rk + u * 16, wv2) for u in range(uk)]
            rl += [lambda u=u: _relayout16(wq_v, g, rq + u * 16, wq2) for u in range(uq)]
            return rl

        def body(p, first=False, last=False):
            fA = proj_pieces(2 * p + 1, qb, kb, vb)
            fB = [] if last else proj_pieces(2 * p + 2, qa, ka, va)
            if first:
                rl = rl_pieces(1 if not dynrl else p + 1, 0, 0, DC // 16, M // 16) if firstrl else []

                def cond_wait():
                    @pl.when(pidx[0] == 0)
                    def _():
                        wait_g1()
                fB = ([] if earlywait else [cond_wait]) + _spread(fB, rl)
                fA = fA[:len(fA) // 2] + [start_mlp_dmas] + fA[len(fA) // 2:] if dma_at == 0 else fA
            if last:
                ob = dict(desc=list(range(ns))[::-1], asc=list(range(ns)), mount=None)[lastorder]
                unified(2 * p, 2 * p + 1, fA, fB, seqB=lastseq, orderB=ob)
            else:
                unified(2 * p, 2 * p + 1, fA, fB)

        def opq(v):
            if not opaque:
                return v
            pidx[0] = v
            return pidx[0]

        with scope("main_loop"):
            if peel == True:
                if earlywait:
                    with scope("p_g1"):
                        wait_g1()
                with scope("m_first"):
                    body(opq(0), first=True)
                start_mlp_dmas()
                with scope("m_loop"):
                    lax.fori_loop(1, H // 2 - 1, lambda p, c: (body(p), c)[1], 0)
                with scope("m_last"):
                    body(opq(H // 2 - 1) if opq_last else H // 2 - 1, last=True)
            else:
                NCH = 6
                uk = -(-(DC // 16) // NCH)
                uq = -(-(M // 16) // NCH)

                def pair_body(p, _):
                    @pl.when(p == 1)
                    def _():
                        wait_g1()
                        start_mlp_dmas()
                    g = jnp.minimum(p, 1)
                    ch = jnp.clip(p - 1, 0, NCH - 1)
                    rk = jnp.minimum(ch * uk, DC // 16 - uk) * 16
                    rq = jnp.minimum(ch * uq, M // 16 - uq) * 16
                    rl = rl_pieces(g, rk, rq, uk, uq)
                    fA = proj_pieces(2 * p + 1, qb, kb, vb)
                    fB = proj_pieces(jnp.minimum(2 * p + 2, H - 1), qa, ka, va)
                    hf = len(rl) // 2
                    unified(2 * p, 2 * p + 1, _spread(fA, rl[:hf]), _spread(fB, rl[hf:]))
                    return 0
                if peel == "last":
                    with scope("m_loop"):
                        lax.fori_loop(0, H // 2 - 1, pair_body, 0)
                    with scope("m_last"):
                        body(H // 2 - 1, last=True)
                else:
                    lax.fori_loop(0, H // 2, pair_body, 0)

        if dma_at < 0:
            for q in (c_wm1, c_wo, c_w1, c_w2, c_w3, c_w4):
                q.start()
        with scope("mod2"):
            c_wm1.wait()
            mod_s[:, 2 * M:6 * M] = _dot(sc, wmod_v[:, 2 * M:6 * M])
            c_wo.wait()
            c_w1.wait()
        ga = mod_s[:, 2 * M:3 * M]
        sb = mod_s[:, 3 * M:4 * M]
        cb = mod_s[:, 4 * M:5 * M]
        gb = mod_s[:, 5 * M:6 * M]
        zpad = jnp.zeros((8, M), F32)
        t_s[0:8, :] = zpad
        t_s[S + 8:S + 16, :] = zpad
        G = M // 4
        offs = (-1, 1, -2, 2)
        nsub = rb // sub

        def X(r, n):
            acc = jnp.zeros((n, M), F32)
            for hd in range(H):
                acc += _dot(ctx_s[hd, pl.ds(_al(r, 16), n), :], wo_v[hd * D:(hd + 1) * D, :])
            xa = x_v[pl.ds(_al(r, 16), n), :].astype(F32) + ga * acc
            xa_s[pl.ds(_al(r, 8), n), :] = xa
            return xa

        def Y1(r, n, xa):
            hb = _ln(xa) * (1.0 + cb) + sb
            hb_s[pl.ds(_al(r, 8), n), :] = hb
            return _ln(hb).astype(BF)

        def Y2(r, n, hl):
            t_s[pl.ds(_al(r + 8, 8), n), :] = _gelu(_dot(hl, w1_v[...]))

        def Z1(r, n):
            lane = lax.broadcasted_iota(jnp.int32, (n, 128), 1)
            cols = []
            for ct in range(M // 128):
                g_lo = (ct * 128) // G
                g_hi = (ct * 128 + 127) // G
                w = t_s[pl.ds(_al(r, 8), n + 16), ct * 128:(ct + 1) * 128]
                a = w[8 + offs[g_lo]:8 + offs[g_lo] + n]
                if g_hi != g_lo:
                    b = w[8 + offs[g_hi]:8 + offs[g_hi] + n]
                    a = jnp.where(lane < (g_hi * G - ct * 128), a, b)
                cols.append(a)
            gsh = jnp.concatenate(cols, axis=1).astype(BF)
            return hb_s[pl.ds(_al(r, 8), n), :] + _dot(gsh, w2_v[...])

        def Z4(r, n, y1, u):
            y2 = y1 + _dot(u, w4_v[...])
            ostage[pl.ds(_al(r, 16), n), :] = (xa_s[pl.ds(_al(r, 8), n), :] + gb * y2).astype(BF)
            pltpu.make_async_copy(ostage.at[pl.ds(_al(r, 16), n), :], out_hbm.at[pl.ds(_al(r, 16), n), :],
                                  osem.at[0]).start()

        def mlp1(i, _):
            r = i * rb
            xs = [None] * nsub
            hl = [None] * nsub
            for k in range(nsub + 2):
                if k < nsub:
                    xs[k] = X(r + k * sub, sub)
                if 0 <= k - 2 < nsub:
                    Y2(r + (k - 2) * sub, sub, hl[k - 2])
                if 0 <= k - 1 < nsub:
                    hl[k - 1] = Y1(r + (k - 1) * sub, sub, xs[k - 1])
            return 0
        with scope("mlp1"):
            lax.fori_loop(0, S // rb, mlp1, 0)

        c_w2.wait()
        c_w3.wait()
        c_w4.wait()

        def mlp2(i, _):
            r = i * rb
            y = [None] * nsub
            l = [None] * nsub
            u = [None] * nsub
            for k in range(nsub + 3):
                if k < nsub:
                    y[k] = Z1(r + k * sub, sub)
                if 0 <= k - 3 < nsub:
                    Z4(r + (k - 3) * sub, sub, y[k - 3], u[k - 3])
                if 0 <= k - 2 < nsub:
                    u[k - 2] = _gelu(_dot_nt(l[k - 2], w3_v[...])).astype(BF)
                if 0 <= k - 1 < nsub:
                    l[k - 1] = _ln(y[k - 1]).astype(BF)
            return 0
        with scope("mlp2"):
            lax.fori_loop(0, S // rb, mlp2, 0)
        pltpu.make_async_copy(ostage, out_hbm, osem.at[0]).wait()

    shapes = dict(
        x_v=((S, M), BF), ckv_v=((S, DC), BF),
        wq_v=((2, M, GH, D), BF), wk_v=((2, DC, GH, D), BF), wv_v=((2, DC, GH, D), BF),
        wo_v=((H * D, M), BF), w1_v=((M, M), BF), w2_v=((M, M), BF), w3_v=((F, M), BF), w4_v=((F, M), BF),
        c_v=((1, M), BF), wmod_v=((M, 6 * M), BF), h1_s=((S, M), BF),
        wq2=((H, M, D), BF), wk2=((H, DC, D), BF), wv2=((H, DC, D), BF), ctx_s=((H + 6, S, D), BF),
        xa_s=((S, M), F32), hb_s=((S, M), F32), t_s=((S + 16, M), F32), mod_s=((1, 6 * M), F32),
        ostage=((S, M), BF))
    for n in names:
        if n.startswith("pad"):
            shapes[n] = ((int(n[3:]), 128), F32)
    scratch = [pltpu.VMEM(*shapes[n]) for n in names] + [
        pltpu.SemaphoreType.DMA((16,)), pltpu.SemaphoreType.DMA((nx,)), pltpu.SemaphoreType.DMA((1,)),
        pltpu.SemaphoreType.DMA((nck,)), pltpu.SMEM((1,), jnp.int32)]

    @jax.jit
    def fn(A_x, A_c_kv, A_w_q, A_w_uk, A_w_uv, A_w_o, B_x, B_w1, B_w2, B_w3, B_w4, c, w_mod):
        del B_x
        hbm = pl.BlockSpec(memory_space=pltpu.HBM)
        out = pl.pallas_call(
            kernel,
            out_shape=jax.ShapeDtypeStruct((S, M), BF),
            in_specs=[hbm] * 12,
            out_specs=hbm,
            scratch_shapes=scratch,
            compiler_params=pltpu.CompilerParams(vmem_limit_bytes=vmem_mb * 1024 * 1024, flags=flags),
        )(A_x.reshape(S, M), A_c_kv.reshape(S, DC), A_w_q, A_w_uk, A_w_uv, A_w_o.reshape(H * D, M),
          B_w1, B_w2, B_w3.T, B_w4, c, w_mod)
        return out.reshape(1, S, M)
    return fn


_kernel = make(peel='last')


def pallas_adaLN_cond__compressed_kv_cla__mixer_s_mlp__prompt_kernel(
    A_x, A_c_kv, A_w_q, A_w_uk, A_w_uv, A_w_o, B_x, B_w1, B_w2, B_w3, B_w4, c, w_mod
):
    return _kernel(A_x, A_c_kv, A_w_q, A_w_uk, A_w_uv, A_w_o, B_x, B_w1, B_w2, B_w3, B_w4, c, w_mod)
```

```python
import math
import jax
import jax.numpy as jnp
from jax import lax
import jax.experimental.pallas as pl
import jax.experimental.pallas.tpu as pltpu

S, M, DC, H, D, F = 2048, 640, 512, 32, 128, 1728
LOG2E = math.log2(math.e)
NEG = -1e9 * LOG2E
QSCALE = D ** -0.5 * LOG2E
BF = jnp.bfloat16
F32 = jnp.float32
U32 = jnp.uint32
GH = 16
BQ = 128


def _ln(x):
    m = jnp.mean(x, axis=-1, keepdims=True)
    d = x - m
    v = jnp.mean(d * d, axis=-1, keepdims=True)
    return d * lax.rsqrt(v + 1e-5)


def _gelu(x):
    k0 = math.sqrt(2.0 / math.pi)
    return 0.5 * x * (1.0 + jnp.tanh(k0 * (x + 0.044715 * (x * x * x))))


def _dot(a, b):
    return jnp.dot(a, b, preferred_element_type=F32)


def _dot_nt(a, b):
    return lax.dot_general(a, b, (((1,), (1,)), ((), ())), preferred_element_type=F32)


def _al(r, n):
    return r if isinstance(r, int) else pl.multiple_of(r, n)


def _transpose8(vs):
    sl = lax.broadcasted_iota(jnp.int32, vs[0].shape, 1)
    for d in (4, 2, 1):
        msk = (sl & d) == 0
        nv = list(vs)
        for i in range(8):
            if i & d:
                continue
            a, b = vs[i], vs[i + d]
            nv[i] = jnp.where(msk, a, pltpu.roll(b, d, 1))
            nv[i + d] = jnp.where(msk, pltpu.roll(a, 8 - d, 1), b)
        vs = nv
    return vs


def _relayout16(raw, g, r0, dst):
    b = raw[g, pl.ds(_al(r0, 16), 16), :, :].reshape(8, 2, 8, 128)
    vs = _transpose8([b[i] for i in range(8)])
    r2 = pl.ds(_al(r0 // 2, 8), 8)
    for j in range(8):
        e, o = vs[j][0], vs[j][1]
        dst[g * GH + 2 * j, r2, :] = (e & jnp.uint32(0xFFFF)) | (o << 16)
        dst[g * GH + 2 * j + 1, r2, :] = (e >> 16) | (o & jnp.uint32(0xFFFF0000))


def _spread(a, b):
    out = []
    nb = 0
    for i, x in enumerate(a):
        out.append(x)
        while nb < len(b) and (nb + 1) * len(a) <= (i + 1) * (len(b) + 0):
            out.append(b[nb])
            nb += 1
    out.extend(b[nb:])
    return out


def make(rb=512, sub=128, vmem_mb=110, order="mount", pc=128, fillpos="after", scopes=False, nx=4, pro=0, rlw="when", dma_at=1, perm=("ckv_v", "h1_s", "wq2", "wk2", "wv2", "ctx_s"), seq="PFQ", div="newton", peel="last", nck=4, opaque=True, xfill=False, sub1=64, onlypro=False, ann=False, rlpos="all", nch=6, rlu=8, pq=512, firstrl=True, dynrl=False, earlywait=False, lastseq="QP", lastorder="mount", opq_last=False, flags=None):
    ns = S // BQ
    import contextlib
    scope = jax.named_scope if scopes else (lambda name: contextlib.nullcontext())

    names = ["x_v", "ckv_v", "wq_v", "wk_v", "wv_v", "wo_v", "w1_v", "w2_v", "w3_v", "w4_v", "c_v", "wmod_v",
             "h1_s", "wq2", "wk2", "wv2", "ctx_s", "xa_s", "hb_s", "t_s", "mod_s", "ostage"]
    if perm is not None:
        names = list(perm) + [n for n in names if n not in perm]

    def kernel(x_hbm, ckv_hbm, wq_hbm, wk_hbm, wv_hbm, wo_hbm, w1_hbm, w2_hbm, w3_hbm, w4_hbm,
               c_hbm, wmod_hbm, out_hbm, *scr):
        R = dict(zip(names, scr[:len(names)]))
        sems, xsem, osem, csem, pidx = scr[len(names):]
        x_v, ckv_v, wq_v, wk_v, wv_v, wo_v, w1_v, w2_v, w3_v, w4_v, c_v, wmod_v = [R[n] for n in
            ("x_v", "ckv_v", "wq_v", "wk_v", "wv_v", "wo_v", "w1_v", "w2_v", "w3_v", "w4_v", "c_v", "wmod_v")]
        h1_s, wq2, wk2, wv2, ctx_s, xa_s, hb_s, t_s, mod_s, ostage = [R[n] for n in
            ("h1_s", "wq2", "wk2", "wv2", "ctx_s", "xa_s", "hb_s", "t_s", "mod_s", "ostage")]

        def cp(i, src, dst):
            return pltpu.make_async_copy(src, dst, sems.at[i])

        xr = S // nx
        c_c = cp(0, c_hbm, c_v)
        c_wm0 = cp(1, wmod_hbm.at[:, 0:2 * M], wmod_v.at[:, 0:2 * M])
        c_wk = [cp(4 + g, wk_hbm.at[:, g * GH:(g + 1) * GH, :], wk_v.bitcast(BF).at[g]) for g in range(2)]
        c_wv = [cp(6 + g, wv_hbm.at[:, g * GH:(g + 1) * GH, :], wv_v.bitcast(BF).at[g]) for g in range(2)]
        c_wq = [cp(8 + g, wq_hbm.at[:, g * GH:(g + 1) * GH, :], wq_v.bitcast(BF).at[g]) for g in range(2)]
        c_wm1 = cp(10, wmod_hbm.at[:, 2 * M:6 * M], wmod_v.at[:, 2 * M:6 * M])
        c_wo = cp(11, wo_hbm, wo_v)
        c_w1 = cp(12, w1_hbm, w1_v)
        c_w2 = cp(13, w2_hbm, w2_v)
        c_w3 = cp(14, w3_hbm, w3_v)
        c_w4 = cp(15, w4_hbm, w4_v)

        qa, ka, va, qb, kb, vb = [ctx_s.at[H + i] for i in range(6)]

        def k_piece(h, kd, r0, n):
            kd[r0:r0 + n, :] = _dot(ckv_v[r0:r0 + n, :], pltpu.bitcast(wk2[h], BF)).astype(BF)

        def v_piece(h, vd, r0, n):
            vd[r0:r0 + n, :] = _dot(ckv_v[r0:r0 + n, :], pltpu.bitcast(wv2[h], BF)).astype(BF)

        def q_piece(h, qd, r0, n):
            qd[r0:r0 + n, :] = (_dot(h1_s[r0:r0 + n, :], pltpu.bitcast(wq2[h], BF)) * QSCALE).astype(BF)

        def proj_pieces(h, qd, kd, vd):
            pcs = []
            for r in range(S // pc):
                pcs.append(lambda r=r: k_piece(h, kd, r * pc, pc))
                pcs.append(lambda r=r: v_piece(h, vd, r * pc, pc))
                pcs.append(lambda r=r: q_piece(h, qd, r * pc, pc))
            return pcs

        cr = S // nck

        def x_copy(i):
            r = _al(i * xr, xr)
            return pltpu.make_async_copy(x_hbm.at[pl.ds(r, xr), :], x_v.at[pl.ds(r, xr), :], xsem.at[i])

        def ck_copy(i):
            r = _al(i * cr, cr)
            return pltpu.make_async_copy(ckv_hbm.at[pl.ds(r, cr), :], ckv_v.at[pl.ds(r, cr), :], csem.at[i])

        def loop(n, f):
            lax.fori_loop(0, n, lambda i, c: (f(i), c)[1], 0)

        def relayout_group(raw, g, dst, rows):
            loop(rows // (16 * rlu), lambda i: [_relayout16(raw, g, (i * rlu + u) * 16, dst) for u in range(rlu)])

        def relayout_group0(raw, dst, rows):
            relayout_group(raw, 0, dst, rows)

        def proj_chunk(src, w, dst, r, n, scale=None):
            y = _dot(src[pl.ds(_al(r, n), n), :], pltpu.bitcast(w[0], BF))
            dst[pl.ds(_al(r, n), n), :] = (y if scale is None else y * scale).astype(BF)

        with scope("p_mod_ln"):
            for q in (c_c, c_wm0):
                q.start()
            loop(nx, lambda i: x_copy(i).start())
            c_wq[0].start()
            c_c.wait()
            c_wm0.wait()
            c_wk[0].start()
            c_wv[0].start()
            cc = c_v[...].astype(F32)
            sc = (cc * jax.nn.sigmoid(cc)).astype(BF)
            mod_s[:, 0:2 * M] = _dot(sc, wmod_v[:, 0:2 * M])
            sa = mod_s[:, 0:M]
            ca = mod_s[:, M:2 * M]

            def ln_chunk(i):
                x_copy(i).wait()
                r = _al(i * xr, xr)
                xx = x_v[pl.ds(r, xr), :].astype(F32)
                h1_s[pl.ds(r, xr), :] = (_ln(xx) * (1.0 + ca) + sa).astype(BF)
            loop(nx, ln_chunk)
        with scope("p_q"):
            c_wq[0].wait()
            loop(nck, lambda i: ck_copy(i).start())
            relayout_group0(wq_v, wq2, M)
            loop(S // pq, lambda i: proj_chunk(h1_s, wq2, qa, i * pq, pq, QSCALE))
        with scope("p_kv"):
            c_wk[0].wait()
            relayout_group0(wk_v, wk2, DC)
            c_wv[0].wait()
            for q in (c_wk[1], c_wv[1], c_wq[1]):
                q.start()
            relayout_group0(wv_v, wv2, DC)

            def kv_chunk(i):
                ck_copy(i).wait()
                proj_chunk(ckv_v, wk2, ka, i * cr, cr)
                proj_chunk(ckv_v, wv2, va, i * cr, cr)
            loop(nck, kv_chunk)

        row_i = lax.broadcasted_iota(jnp.int32, (BQ, BQ), 0)
        col_i = lax.broadcasted_iota(jnp.int32, (BQ, BQ), 1)
        tri = col_i <= row_i

        def qk(i, qs, ks):
            q0 = i * BQ
            s = _dot_nt(qs[q0:q0 + BQ, :], ks[0:q0 + BQ, :])
            sd = jnp.where(tri, s[:, q0:], NEG)
            return jnp.concatenate([s[:, :q0], sd], axis=1) if i > 0 else sd

        def sm(s):
            m = jnp.max(s, axis=1, keepdims=True)
            p = jnp.exp2(s - m)
            l = jnp.sum(p, axis=1, keepdims=True)
            return p.astype(BF), l

        def pv(i, hd, pl_, vs):
            q0 = i * BQ
            p, l = pl_
            o = _dot(p, vs[0:q0 + BQ, :])
            if div == "div":
                o = o / l
            else:
                o = o * (1.0 / l)
            ctx_s[hd, q0:q0 + BQ, :] = o.astype(BF)

        def head_order():
            idx = list(range(ns))
            if order == "desc":
                return idx[::-1]
            if order == "asc":
                return idx
            return idx[0::2] + idx[1::2][::-1]

        def alloc(nf):
            return [(nf * (n + 1)) // ns - (nf * n) // ns for n in range(ns)]

        def unified(hA, hB, fA, fB, seqB=None, orderB=None, perB=None):
            ho = head_order()
            hoB = ho if orderB is None else orderB
            tasks = [(hA, i, qa, ka, va) for i in ho] + [(hB, i, qb, kb, vb) for i in hoB]
            if perB is not None:
                fB = [f for st in perB for f in st]
                alB = [len(st) for st in perB]
            else:
                alB = alloc(len(fB))
            alA = alloc(len(fA))
            nt = len(tasks)
            sv = {0: qk(tasks[0][1], tasks[0][2], tasks[0][3])}
            pvv = {}
            for n in range(nt + 1):
                fl, al = (fA, alA) if n < ns else (fB, alB)
                for ch in (seqB if (seqB and n >= ns) else seq):
                    if ch == "Q" and n + 1 < nt:
                        t = tasks[n + 1]
                        sv[n + 1] = qk(t[1], t[2], t[3])
                    elif ch == "P" and 0 <= n - 1 < nt:
                        t = tasks[n - 1]
                        pv(t[1], t[0], pvv.pop(n - 1), t[4])
                    elif ch == "F" and n < nt:
                        for _ in range(al[n % ns]):
                            fl.pop(0)()
                if n < nt:
                    pvv[n] = sm(sv.pop(n))
            assert not fA and not fB

        def mod_rest():
            c_wm1.wait()
            mod_s[:, 2 * M:6 * M] = _dot(sc, wmod_v[:, 2 * M:6 * M])
            c_wo.wait()
            c_w1.wait()
            zpad = jnp.zeros((8, M), F32)
            t_s[0:8, :] = zpad
            t_s[S + 8:S + 16, :] = zpad

        def modp(j, c0=0, c1=M):
            return mod_s[:, j * M + c0:j * M + c1]

        G = M // 4
        offs = (-1, 1, -2, 2)

        def X(r, n):
            acc = jnp.zeros((n, M), F32)
            for hd in range(H):
                acc += _dot(ctx_s[hd, pl.ds(_al(r, 16), n), :], wo_v[hd * D:(hd + 1) * D, :])
            xa = x_v[pl.ds(_al(r, 16), n), :].astype(F32) + modp(2) * acc
            xa_s[pl.ds(_al(r, 8), n), :] = xa
            return xa

        def Y1(r, n, xa):
            hb = _ln(xa) * (1.0 + modp(4)) + modp(3)
            hb_s[pl.ds(_al(r, 8), n), :] = hb
            return _ln(hb).astype(BF)

        def Y2(r, n, hl):
            t_s[pl.ds(_al(r + 8, 8), n), :] = _gelu(_dot(hl, w1_v[...]))

        def Z1(r, n):
            lane = lax.broadcasted_iota(jnp.int32, (n, 128), 1)
            cols = []
            for ct in range(M // 128):
                g_lo = (ct * 128) // G
                g_hi = (ct * 128 + 127) // G
                w = t_s[pl.ds(_al(r, 8), n + 16), ct * 128:(ct + 1) * 128]
                a = w[8 + offs[g_lo]:8 + offs[g_lo] + n]
                if g_hi != g_lo:
                    b = w[8 + offs[g_hi]:8 + offs[g_hi] + n]
                    a = jnp.where(lane < (g_hi * G - ct * 128), a, b)
                cols.append(a)
            gsh = jnp.concatenate(cols, axis=1).astype(BF)
            return hb_s[pl.ds(_al(r, 8), n), :] + _dot(gsh, w2_v[...])

        def Z4(r, n, y1, u):
            y2 = y1 + _dot(u, w4_v[...])
            ostage[pl.ds(_al(r, 16), n), :] = (xa_s[pl.ds(_al(r, 8), n), :] + modp(5) * y2).astype(BF)
            pltpu.make_async_copy(ostage.at[pl.ds(_al(r, 16), n), :], out_hbm.at[pl.ds(_al(r, 16), n), :],
                                  osem.at[0]).start()

        def Xc(r, n, ct):
            cs = slice(ct * 128, (ct + 1) * 128)
            acc = jnp.zeros((n, 128), F32)
            for hd in range(H):
                acc += _dot(ctx_s[hd, pl.ds(_al(r, 16), n), :], wo_v[hd * D:(hd + 1) * D, cs])
            xa_s[pl.ds(_al(r, 8), n), cs] = x_v[pl.ds(_al(r, 16), n), cs].astype(F32) + modp(2, ct * 128, (ct + 1) * 128) * acc

        def start_mlp_dmas():
            for q in (c_wm1, c_wo, c_w1, c_w2, c_w3, c_w4):
                q.start()

        def wait_g1():
            c_wk[1].wait()
            c_wv[1].wait()
            c_wq[1].wait()

        def rl_pieces(g, rk, rq, uk, uq, wk2=wk2, wv2=wv2, wq2=wq2):
            if ann:
                wk2, wv2, wq2 = [pltpu.annotate(r, no_hazard_no_deps=True) for r in (wk2, wv2, wq2)]
            rl = [lambda u=u: _relayout16(wk_v, g, rk + u * 16, wk2) for u in range(uk)]
            rl += [lambda u=u: _relayout16(wv_v, g, rk + u * 16, wv2) for u in range(uk)]
            rl += [lambda u=u: _relayout16(wq_v, g, rq + u * 16, wq2) for u in range(uq)]
            return rl

        def place(a, b):
            n = len(a)
            if rlpos == "all":
                return _spread(a, b)
            if rlpos == "mid":
                return a[:n // 4] + _spread(a[n // 4:3 * n // 4], b) + a[3 * n // 4:]
            if rlpos == "ends":
                h = len(b) // 2
                return _spread(a[:n // 4], b[:h]) + a[n // 4:3 * n // 4] + _spread(a[3 * n // 4:], b[h:])
            if rlpos == "first":
                return _spread(a[:n // 2], b) + a[n // 2:]
            if rlpos == "last":
                return a[:n // 2] + _spread(a[n // 2:], b)

        def body(p, first=False, last=False):
            fA = proj_pieces(2 * p + 1, qb, kb, vb)
            fB = [] if last else proj_pieces(2 * p + 2, qa, ka, va)
            if first:
                rl = rl_pieces(1 if not dynrl else p + 1, 0, 0, DC // 16, M // 16) if firstrl else []

                def cond_wait():
                    @pl.when(pidx[0] == 0)
                    def _():
                        wait_g1()
                fB = ([] if earlywait else [cond_wait]) + _spread(fB, rl)
                fA = fA[:len(fA) // 2] + [start_mlp_dmas] + fA[len(fA) // 2:] if dma_at == 0 else fA
            if last:
                mod_rest()
                if xfill:
                    per = [[] for _ in range(ns)]
                    pcs = [(k, ct) for k in range(rb // BQ) for ct in range(M // 128)]
                    st = 1
                    for j, (k, ct) in enumerate(pcs):
                        st = max(k + 1, 1 + (j * (ns - 1)) // len(pcs))
                        per[st].append(lambda k=k, ct=ct: Xc(k * BQ, BQ, ct))
                    unified(2 * p, 2 * p + 1, fA, None, seqB=seq, orderB=list(range(ns)), perB=per)
                    return
                ob = dict(desc=list(range(ns))[::-1], asc=list(range(ns)), mount=None)[lastorder]
                unified(2 * p, 2 * p + 1, fA, fB, seqB=lastseq, orderB=ob)
            else:
                unified(2 * p, 2 * p + 1, fA, fB)

        def opq(v):
            if not opaque:
                return v
            pidx[0] = v
            return pidx[0]

        if onlypro:
            for q in (c_wk[1], c_wv[1], c_wq[1]):
                q.wait()
            return
        with scope("main_loop"):
            if peel == True:
                if earlywait:
                    with scope("p_g1"):
                        wait_g1()
                with scope("m_first"):
                    body(opq(0), first=True)
                start_mlp_dmas()
                with scope("m_loop"):
                    lax.fori_loop(1, H // 2 - 1, lambda p, c: (body(p), c)[1], 0)
                with scope("m_last"):
                    body(opq(H // 2 - 1) if opq_last else H // 2 - 1, last=True)
            else:
                NCH = nch
                uk = -(-(DC // 16) // NCH)
                uq = -(-(M // 16) // NCH)

                def pair_body(p, _):
                    @pl.when(p == 1)
                    def _():
                        wait_g1()
                        start_mlp_dmas()
                        if rlw == "when":
                            relayout_group(wk_v, 1, wk2, DC)
                            relayout_group(wv_v, 1, wv2, DC)
                            relayout_group(wq_v, 1, wq2, M)
                    g = jnp.minimum(p, 1)
                    ch = jnp.clip(p - 1, 0, NCH - 1)
                    rk = jnp.minimum(ch * uk, DC // 16 - uk) * 16
                    rq = jnp.minimum(ch * uq, M // 16 - uq) * 16
                    rl = rl_pieces(g, rk, rq, uk, uq) if rlw != "when" else []
                    fA = proj_pieces(2 * p + 1, qb, kb, vb)
                    fB = proj_pieces(jnp.minimum(2 * p + 2, H - 1), qa, ka, va)
                    hf = len(rl) // 2
                    unified(2 * p, 2 * p + 1, place(fA, rl[:hf]), place(fB, rl[hf:]))
                    return 0
                if peel == "last":
                    with scope("m_loop"):
                        lax.fori_loop(0, H // 2 - 1, pair_body, 0)
                    with scope("m_last"):
                        body(H // 2 - 1, last=True)
                else:
                    lax.fori_loop(0, H // 2, pair_body, 0)

        def mlp1(i, _, with_x=True):
            r = i * rb
            n1 = rb // sub1
            if not xfill:
                xs = [None] * n1
                hl = [None] * n1
                for k in range(n1 + 2):
                    if k < n1:
                        xs[k] = X(r + k * sub1, sub1)
                    if 0 <= k - 2 < n1:
                        Y2(r + (k - 2) * sub1, sub1, hl[k - 2])
                    if 0 <= k - 1 < n1:
                        hl[k - 1] = Y1(r + (k - 1) * sub1, sub1, xs[k - 1])
                return 0
            xs = [xa_s[pl.ds(_al(r + k * sub1, 8), sub1), :] for k in range(n1)]
            hl = [None] * n1
            for k in range(n1 + 1):
                if k < n1:
                    hl[k] = Y1(r + k * sub1, sub1, xs[k])
                    if with_x:
                        X(r + rb + k * sub1, sub1)
                if 0 <= k - 1 < n1:
                    Y2(r + (k - 1) * sub1, sub1, hl[k - 1])
            return 0
        with scope("mlp1"):
            if xfill:
                lax.fori_loop(0, S // rb - 1, mlp1, 0)
                mlp1(S // rb - 1, 0, with_x=False)
            else:
                lax.fori_loop(0, S // rb, mlp1, 0)

        c_w2.wait()
        c_w3.wait()
        c_w4.wait()

        def mlp2(i, _):
            r = i * rb
            nsub = rb // sub
            y = [None] * nsub
            l = [None] * nsub
            u = [None] * nsub
            for k in range(nsub + 3):
                if k < nsub:
                    y[k] = Z1(r + k * sub, sub)
                if 0 <= k - 3 < nsub:
                    Z4(r + (k - 3) * sub, sub, y[k - 3], u[k - 3])
                if 0 <= k - 2 < nsub:
                    u[k - 2] = _gelu(_dot_nt(l[k - 2], w3_v[...])).astype(BF)
                if 0 <= k - 1 < nsub:
                    l[k - 1] = _ln(y[k - 1]).astype(BF)
            return 0
        with scope("mlp2"):
            lax.fori_loop(0, S // rb, mlp2, 0)
        pltpu.make_async_copy(ostage, out_hbm, osem.at[0]).wait()

    shapes = dict(
        x_v=((S, M), BF), ckv_v=((S, DC), BF),
        wq_v=((2, M, GH // 2, D), U32), wk_v=((2, DC, GH // 2, D), U32), wv_v=((2, DC, GH // 2, D), U32),
        wo_v=((H * D, M), BF), w1_v=((M, M), BF), w2_v=((M, M), BF), w3_v=((F, M), BF), w4_v=((F, M), BF),
        c_v=((1, M), BF), wmod_v=((M, 6 * M), BF), h1_s=((S, M), BF),
        wq2=((H, M // 2, D), U32), wk2=((H, DC // 2, D), U32), wv2=((H, DC // 2, D), U32), ctx_s=((H + 6, S, D), BF),
        xa_s=((S, M), F32), hb_s=((S, M), F32), t_s=((S + 16, M), F32), mod_s=((1, 6 * M), F32),
        ostage=((S, M), BF))
    for n in names:
        if n.startswith("pad"):
            shapes[n] = ((int(n[3:]), 128), F32)
    scratch = [pltpu.VMEM(*shapes[n]) for n in names] + [
        pltpu.SemaphoreType.DMA((16,)), pltpu.SemaphoreType.DMA((nx,)), pltpu.SemaphoreType.DMA((1,)),
        pltpu.SemaphoreType.DMA((nck,)), pltpu.SMEM((1,), jnp.int32)]

    @jax.jit
    def fn(A_x, A_c_kv, A_w_q, A_w_uk, A_w_uv, A_w_o, B_x, B_w1, B_w2, B_w3, B_w4, c, w_mod):
        del B_x
        hbm = pl.BlockSpec(memory_space=pltpu.HBM)
        out = pl.pallas_call(
            kernel,
            out_shape=jax.ShapeDtypeStruct((S, M), BF),
            in_specs=[hbm] * 12,
            out_specs=hbm,
            scratch_shapes=scratch,
            compiler_params=pltpu.CompilerParams(vmem_limit_bytes=vmem_mb * 1024 * 1024, flags=flags),
        )(A_x.reshape(S, M), A_c_kv.reshape(S, DC), A_w_q, A_w_uk, A_w_uv, A_w_o.reshape(H * D, M),
          B_w1, B_w2, B_w3.T, B_w4, c, w_mod)
        return out.reshape(1, S, M)
    return fn


_kernel = make()


def pallas_adaLN_cond__compressed_kv_cla__mixer_s_mlp__prompt_kernel(
    A_x, A_c_kv, A_w_q, A_w_uk, A_w_uv, A_w_o, B_x, B_w1, B_w2, B_w3, B_w4, c, w_mod
):
    return _kernel(A_x, A_c_kv, A_w_q, A_w_uk, A_w_uv, A_w_o, B_x, B_w1, B_w2, B_w3, B_w4, c, w_mod)
```

```python
import math

import jax
import jax.numpy as jnp
from jax import lax
import jax.experimental.pallas as pl
import jax.experimental.pallas.tpu as pltpu

S, M, DC, H, D, F = 2048, 640, 512, 32, 128, 1728
LOG2E = math.log2(math.e)
NEG = -1e9 * LOG2E
QSCALE = D ** -0.5 * LOG2E
BF = jnp.bfloat16
F32 = jnp.float32
U32 = jnp.uint32
GH = 16
BQ = 128
NS = S // BQ
PC = 128
RB = 512
SUB1, SUB2 = 64, 128
NX = 4
RLU = 8


def _ln(x):
    m = jnp.mean(x, axis=-1, keepdims=True)
    d = x - m
    v = jnp.mean(d * d, axis=-1, keepdims=True)
    return d * lax.rsqrt(v + 1e-5)


def _gelu(x):
    k0 = math.sqrt(2.0 / math.pi)
    return 0.5 * x * (1.0 + jnp.tanh(k0 * (x + 0.044715 * (x * x * x))))


def _dot(a, b):
    return jnp.dot(a, b, preferred_element_type=F32)


def _dot_nt(a, b):
    return lax.dot_general(a, b, (((1,), (1,)), ((), ())), preferred_element_type=F32)


def _al(r, n):
    return r if isinstance(r, int) else pl.multiple_of(r, n)


def _loop(lo, hi, f):
    lax.fori_loop(lo, hi, lambda i, c: (f(i), c)[1], 0)


def _transpose8(vs):
    sl = lax.broadcasted_iota(jnp.int32, vs[0].shape, 1)
    for d in (4, 2, 1):
        msk = (sl & d) == 0
        nv = list(vs)
        for i in range(8):
            if i & d:
                continue
            a, b = vs[i], vs[i + d]
            nv[i] = jnp.where(msk, a, pltpu.roll(b, d, 1))
            nv[i + d] = jnp.where(msk, pltpu.roll(a, 8 - d, 1), b)
        vs = nv
    return vs


def _relayout16(raw, g, r0, dst):
    b = raw[g, pl.ds(_al(r0, 16), 16), :, :].reshape(8, 2, 8, 128)
    vs = _transpose8([b[i] for i in range(8)])
    r2 = pl.ds(_al(r0 // 2, 8), 8)
    for j in range(8):
        e, o = vs[j][0], vs[j][1]
        dst[g * GH + 2 * j, r2, :] = (e & jnp.uint32(0xFFFF)) | (o << 16)
        dst[g * GH + 2 * j + 1, r2, :] = (e >> 16) | (o & jnp.uint32(0xFFFF0000))


def _kernel(x_hbm, ckv_hbm, wq_hbm, wk_hbm, wv_hbm, wo_hbm, w1_hbm, w2_hbm, w3_hbm, w4_hbm, c_hbm, wmod_hbm,
            out_hbm,
            ckv_v, h1_s, wq2, wk2, wv2, ctx_s, wo_v, x_v, xa_s, hb_s, t_s, w1_v, w2_v, w3_v, w4_v, ostage, mod_s,
            wq_v, wk_v, wv_v, c_v, wmod_v,
            sems, xsem, csem, osem):
    def cp(i, src, dst):
        return pltpu.make_async_copy(src, dst, sems.at[i])

    xr = S // NX
    c_c = cp(0, c_hbm, c_v)
    c_wm0 = cp(1, wmod_hbm.at[:, 0:2 * M], wmod_v.at[:, 0:2 * M])
    c_wm1 = cp(2, wmod_hbm.at[:, 2 * M:6 * M], wmod_v.at[:, 2 * M:6 * M])
    c_wk = [cp(3 + g, wk_hbm.at[:, g * GH:(g + 1) * GH, :], wk_v.bitcast(BF).at[g]) for g in range(2)]
    c_wv = [cp(5 + g, wv_hbm.at[:, g * GH:(g + 1) * GH, :], wv_v.bitcast(BF).at[g]) for g in range(2)]
    c_wq = [cp(7 + g, wq_hbm.at[:, g * GH:(g + 1) * GH, :], wq_v.bitcast(BF).at[g]) for g in range(2)]
    c_wo = cp(9, wo_hbm, wo_v)
    c_w1 = cp(10, w1_hbm, w1_v)
    c_w2 = cp(11, w2_hbm, w2_v)
    c_w3 = cp(12, w3_hbm, w3_v)
    c_w4 = cp(13, w4_hbm, w4_v)

    def x_copy(i):
        r = _al(i * xr, xr)
        return pltpu.make_async_copy(x_hbm.at[pl.ds(r, xr), :], x_v.at[pl.ds(r, xr), :], xsem.at[i])

    def ck_copy(i):
        r = _al(i * xr, xr)
        return pltpu.make_async_copy(ckv_hbm.at[pl.ds(r, xr), :], ckv_v.at[pl.ds(r, xr), :], csem.at[i])

    qa, ka, va, qb, kb, vb = [ctx_s.at[H + i] for i in range(6)]

    def project(src, w, h, dst, r, n, scale=None):
        y = _dot(src[pl.ds(_al(r, n), n), :], pltpu.bitcast(w[h], BF))
        dst[pl.ds(_al(r, n), n), :] = (y if scale is None else y * scale).astype(BF)

    def relayout_group(raw, g, dst, rows):
        _loop(0, rows // (16 * RLU),
              lambda i: [_relayout16(raw, g, (i * RLU + u) * 16, dst) for u in range(RLU)])

    for q in (c_c, c_wm0):
        q.start()
    _loop(0, NX, lambda i: x_copy(i).start())
    c_wq[0].start()
    c_c.wait()
    c_wm0.wait()
    c_wk[0].start()
    c_wv[0].start()
    cc = c_v[...].astype(F32)
    sc = (cc * jax.nn.sigmoid(cc)).astype(BF)
    mod_s[:, 0:2 * M] = _dot(sc, wmod_v[:, 0:2 * M])
    sa = mod_s[:, 0:M]
    ca = mod_s[:, M:2 * M]

    def ln_chunk(i):
        x_copy(i).wait()
        r = _al(i * xr, xr)
        xx = x_v[pl.ds(r, xr), :].astype(F32)
        h1_s[pl.ds(r, xr), :] = (_ln(xx) * (1.0 + ca) + sa).astype(BF)
    _loop(0, NX, ln_chunk)

    c_wq[0].wait()
    _loop(0, NX, lambda i: ck_copy(i).start())
    relayout_group(wq_v, 0, wq2, M)
    _loop(0, NX, lambda i: project(h1_s, wq2, 0, qa, i * xr, xr, QSCALE))
    c_wk[0].wait()
    relayout_group(wk_v, 0, wk2, DC)
    c_wv[0].wait()
    for q in (c_wk[1], c_wv[1], c_wq[1]):
        q.start()
    relayout_group(wv_v, 0, wv2, DC)

    def kv_chunk(i):
        ck_copy(i).wait()
        project(ckv_v, wk2, 0, ka, i * xr, xr)
        project(ckv_v, wv2, 0, va, i * xr, xr)
    _loop(0, NX, kv_chunk)

    tri = lax.broadcasted_iota(jnp.int32, (BQ, BQ), 1) <= lax.broadcasted_iota(jnp.int32, (BQ, BQ), 0)

    def proj_pieces(h, qd, kd, vd):
        pcs = []
        for r in range(S // PC):
            pcs.append(lambda r=r: project(ckv_v, wk2, h, kd, r * PC, PC))
            pcs.append(lambda r=r: project(ckv_v, wv2, h, vd, r * PC, PC))
            pcs.append(lambda r=r: project(h1_s, wq2, h, qd, r * PC, PC, QSCALE))
        return pcs

    def qk(i, qs, ks):
        q0 = i * BQ
        s = _dot_nt(qs[q0:q0 + BQ, :], ks[0:q0 + BQ, :])
        sd = jnp.where(tri, s[:, q0:], NEG)
        return jnp.concatenate([s[:, :q0], sd], axis=1) if i > 0 else sd

    def softmax(s):
        m = jnp.max(s, axis=1, keepdims=True)
        p = jnp.exp2(s - m)
        return p.astype(BF), jnp.sum(p, axis=1, keepdims=True)

    def pv(i, hd, p, l, vs):
        q0 = i * BQ
        o = _dot(p, vs[0:q0 + BQ, :]) * (1.0 / l)
        ctx_s[hd, q0:q0 + BQ, :] = o.astype(BF)

    order = list(range(NS))[0::2] + list(range(NS))[1::2][::-1]

    def share(nf):
        return [(nf * (n + 1)) // NS - (nf * n) // NS for n in range(NS)]

    def head_pair(ha, hb, fa, fb):
        tasks = [(ha, i, qa, ka, va) for i in order] + [(hb, i, qb, kb, vb) for i in order]
        nt = len(tasks)
        quota = share(len(fa)) + share(len(fb))
        scores = {0: qk(*tasks[0][1:4])}
        probs = {}

        def do_q(n):
            if n + 1 < nt:
                scores[n + 1] = qk(*tasks[n + 1][1:4])

        def do_p(n):
            if 0 <= n - 1 < nt:
                hd, i, _, _, vs = tasks[n - 1]
                pv(i, hd, *probs.pop(n - 1), vs)

        for n in range(nt + 1):
            fill = fa if n < NS else fb
            if n < NS or fb:
                do_p(n)
                for _ in range(quota[n] if n < nt else 0):
                    fill.pop(0)()
                do_q(n)
            else:
                do_q(n)
                do_p(n)
            if n < nt:
                probs[n] = softmax(scores.pop(n))

    def pair_body(p):
        @pl.when(p == 1)
        def _():
            for q in (c_wk[1], c_wv[1], c_wq[1]):
                q.wait()
            for q in (c_wm1, c_wo, c_w1, c_w2, c_w3, c_w4):
                q.start()
            relayout_group(wk_v, 1, wk2, DC)
            relayout_group(wv_v, 1, wv2, DC)
            relayout_group(wq_v, 1, wq2, M)
        head_pair(2 * p, 2 * p + 1, proj_pieces(2 * p + 1, qb, kb, vb), proj_pieces(2 * p + 2, qa, ka, va))
    _loop(0, H // 2 - 1, pair_body)

    c_wm1.wait()
    mod_s[:, 2 * M:6 * M] = _dot(sc, wmod_v[:, 2 * M:6 * M])
    c_wo.wait()
    c_w1.wait()
    zpad = jnp.zeros((8, M), F32)
    t_s[0:8, :] = zpad
    t_s[S + 8:S + 16, :] = zpad
    head_pair(H - 2, H - 1, proj_pieces(H - 1, qb, kb, vb), [])

    def modp(j):
        return mod_s[:, j * M:(j + 1) * M]

    def out_proj(r, n):
        acc = jnp.zeros((n, M), F32)
        for hd in range(H):
            acc += _dot(ctx_s[hd, pl.ds(_al(r, 16), n), :], wo_v[hd * D:(hd + 1) * D, :])
        xa = x_v[pl.ds(_al(r, 16), n), :].astype(F32) + modp(2) * acc
        xa_s[pl.ds(_al(r, 8), n), :] = xa
        return xa

    def ada_ln(r, n, xa):
        hb = _ln(xa) * (1.0 + modp(4)) + modp(3)
        hb_s[pl.ds(_al(r, 8), n), :] = hb
        return _ln(hb).astype(BF)

    def mlp1(i):
        r, n = i * RB, RB // SUB1
        xs, hl = [None] * n, [None] * n
        for k in range(n + 2):
            if k < n:
                xs[k] = out_proj(r + k * SUB1, SUB1)
            if 0 <= k - 2 < n:
                t_s[pl.ds(_al(r + (k - 2) * SUB1 + 8, 8), SUB1), :] = _gelu(_dot(hl[k - 2], w1_v[...]))
            if 0 <= k - 1 < n:
                hl[k - 1] = ada_ln(r + (k - 1) * SUB1, SUB1, xs[k - 1])
    _loop(0, S // RB, mlp1)

    c_w2.wait()
    c_w3.wait()
    c_w4.wait()
    G = M // 4
    offs = (-1, 1, -2, 2)

    def shift_proj(r, n):
        lane = lax.broadcasted_iota(jnp.int32, (n, 128), 1)
        cols = []
        for ct in range(M // 128):
            g_lo, g_hi = (ct * 128) // G, (ct * 128 + 127) // G
            w = t_s[pl.ds(_al(r, 8), n + 16), ct * 128:(ct + 1) * 128]
            a = w[8 + offs[g_lo]:8 + offs[g_lo] + n]
            if g_hi != g_lo:
                a = jnp.where(lane < (g_hi * G - ct * 128), a, w[8 + offs[g_hi]:8 + offs[g_hi] + n])
            cols.append(a)
        g = jnp.concatenate(cols, axis=1).astype(BF)
        return hb_s[pl.ds(_al(r, 8), n), :] + _dot(g, w2_v[...])

    def finish(r, n, y1, u):
        y2 = y1 + _dot(u, w4_v[...])
        rows = pl.ds(_al(r, 16), n)
        ostage[rows, :] = (xa_s[pl.ds(_al(r, 8), n), :] + modp(5) * y2).astype(BF)
        pltpu.make_async_copy(ostage.at[rows, :], out_hbm.at[rows, :], osem.at[0]).start()

    def mlp2(i):
        r, n = i * RB, RB // SUB2
        y, l, u = [None] * n, [None] * n, [None] * n
        for k in range(n + 3):
            if k < n:
                y[k] = shift_proj(r + k * SUB2, SUB2)
            if 0 <= k - 3 < n:
                finish(r + (k - 3) * SUB2, SUB2, y[k - 3], u[k - 3])
            if 0 <= k - 2 < n:
                u[k - 2] = _gelu(_dot_nt(l[k - 2], w3_v[...])).astype(BF)
            if 0 <= k - 1 < n:
                l[k - 1] = _ln(y[k - 1]).astype(BF)
    _loop(0, S // RB, mlp2)
    pltpu.make_async_copy(ostage, out_hbm, osem.at[0]).wait()


@jax.jit
def pallas_adaLN_cond__compressed_kv_cla__mixer_s_mlp__prompt_kernel(
    A_x, A_c_kv, A_w_q, A_w_uk, A_w_uv, A_w_o, B_x, B_w1, B_w2, B_w3, B_w4, c, w_mod
):
    del B_x
    vmem = pltpu.VMEM
    scratch = [
        vmem((S, DC), BF), vmem((S, M), BF),
        vmem((H, M // 2, D), U32), vmem((H, DC // 2, D), U32), vmem((H, DC // 2, D), U32),
        vmem((H + 6, S, D), BF),
        vmem((H * D, M), BF), vmem((S, M), BF),
        vmem((S, M), F32), vmem((S, M), F32), vmem((S + 16, M), F32),
        vmem((M, M), BF), vmem((M, M), BF), vmem((F, M), BF), vmem((F, M), BF),
        vmem((S, M), BF), vmem((1, 6 * M), F32),
        vmem((2, M, GH // 2, D), U32), vmem((2, DC, GH // 2, D), U32), vmem((2, DC, GH // 2, D), U32),
        vmem((1, M), BF), vmem((M, 6 * M), BF),
        pltpu.SemaphoreType.DMA((14,)), pltpu.SemaphoreType.DMA((NX,)), pltpu.SemaphoreType.DMA((NX,)),
        pltpu.SemaphoreType.DMA((1,)),
    ]
    hbm = pl.BlockSpec(memory_space=pltpu.HBM)
    out = pl.pallas_call(
        _kernel,
        out_shape=jax.ShapeDtypeStruct((S, M), BF),
        in_specs=[hbm] * 12,
        out_specs=hbm,
        scratch_shapes=scratch,
        compiler_params=pltpu.CompilerParams(vmem_limit_bytes=110 * 1024 * 1024),
    )(A_x.reshape(S, M), A_c_kv.reshape(S, DC), A_w_q, A_w_uk, A_w_uv, A_w_o.reshape(H * D, M),
      B_w1, B_w2, B_w3.T, B_w4, c, w_mod)
    return out.reshape(1, S, M)
```

```python
import math

import jax
import jax.numpy as jnp
from jax import lax
import jax.experimental.pallas as pl
import jax.experimental.pallas.tpu as pltpu

S, M, DC, H, D, F = 2048, 640, 512, 32, 128, 1728
LOG2E = math.log2(math.e)
NEG = -1e9 * LOG2E
QSCALE = D ** -0.5 * LOG2E
BF = jnp.bfloat16
F32 = jnp.float32
U32 = jnp.uint32
GH = 16
BQ = 128
NS = S // BQ
PC = 128
RB = 512
SUB1, SUB2 = 64, 128
NX = 4
RLU = 8


def _ln(x):
    m = jnp.mean(x, axis=-1, keepdims=True)
    d = x - m
    v = jnp.mean(d * d, axis=-1, keepdims=True)
    return d * lax.rsqrt(v + 1e-5)


def _gelu(x):
    k0 = math.sqrt(2.0 / math.pi)
    return 0.5 * x * (1.0 + jnp.tanh(k0 * (x + 0.044715 * (x * x * x))))


def _dot(a, b):
    return jnp.dot(a, b, preferred_element_type=F32)


def _dot_nt(a, b):
    return lax.dot_general(a, b, (((1,), (1,)), ((), ())), preferred_element_type=F32)


def _al(r, n):
    return r if isinstance(r, int) else pl.multiple_of(r, n)


def _loop(lo, hi, f):
    lax.fori_loop(lo, hi, lambda i, c: (f(i), c)[1], 0)


def _transpose8(vs):
    sl = lax.broadcasted_iota(jnp.int32, vs[0].shape, 1)
    for d in (4, 2, 1):
        msk = (sl & d) == 0
        nv = list(vs)
        for i in range(8):
            if i & d:
                continue
            a, b = vs[i], vs[i + d]
            nv[i] = jnp.where(msk, a, pltpu.roll(b, d, 1))
            nv[i + d] = jnp.where(msk, pltpu.roll(a, 8 - d, 1), b)
        vs = nv
    return vs


def _relayout16(raw, g, r0, dst):
    b = pltpu.bitcast(raw[g, pl.ds(_al(r0, 16), 16), :, :], U32)
    b = b.reshape(8, 2, 8, 128)
    vs = _transpose8([b[i] for i in range(8)])
    r2 = pl.ds(_al(r0 // 2, 8), 8)
    for j in range(8):
        e, o = vs[j][0], vs[j][1]
        dst[g * GH + 2 * j, r2, :] = (e & jnp.uint32(0xFFFF)) | (o << 16)
        dst[g * GH + 2 * j + 1, r2, :] = (e >> 16) | (o & jnp.uint32(0xFFFF0000))


def _kernel(x_hbm, ckv_hbm, wq_hbm, wk_hbm, wv_hbm, wo_hbm, w1_hbm, w2_hbm, w3_hbm, w4_hbm, c_hbm, wmod_hbm,
            out_hbm,
            ckv_v, h1_s, wq2, wk2, wv2, ctx_s, wo_v, x_v, xa_s, hb_s, t_s, w1_v, w2_v, w3_v, w4_v, ostage, mod_s,
            wq_v, wk_v, wv_v, c_v, wmod_v,
            sems, xsem, csem, osem):
    def cp(i, src, dst):
        return pltpu.make_async_copy(src, dst, sems.at[i])

    xr = S // NX
    c_c = cp(0, c_hbm, c_v)
    c_wm0 = cp(1, wmod_hbm.at[:, 0:2 * M], wmod_v.at[:, 0:2 * M])
    c_wm1 = cp(2, wmod_hbm.at[:, 2 * M:6 * M], wmod_v.at[:, 2 * M:6 * M])
    c_wk = [cp(3 + g, wk_hbm.at[:, g * GH:(g + 1) * GH, :], wk_v.at[g]) for g in range(2)]
    c_wv = [cp(5 + g, wv_hbm.at[:, g * GH:(g + 1) * GH, :], wv_v.at[g]) for g in range(2)]
    c_wq = [cp(7 + g, wq_hbm.at[:, g * GH:(g + 1) * GH, :], wq_v.at[g]) for g in range(2)]
    c_wo = cp(9, wo_hbm, wo_v)
    c_w1 = cp(10, w1_hbm, w1_v)
    c_w2 = cp(11, w2_hbm, w2_v)
    c_w3 = cp(12, w3_hbm, w3_v)
    c_w4 = cp(13, w4_hbm, w4_v)

    def x_copy(i):
        r = _al(i * xr, xr)
        return pltpu.make_async_copy(x_hbm.at[pl.ds(r, xr), :], x_v.at[pl.ds(r, xr), :], xsem.at[i])

    def ck_copy(i):
        r = _al(i * xr, xr)
        return pltpu.make_async_copy(ckv_hbm.at[pl.ds(r, xr), :], ckv_v.at[pl.ds(r, xr), :], csem.at[i])

    qa, ka, va, qb, kb, vb = [ctx_s.at[H + i] for i in range(6)]

    def project(src, w, h, dst, r, n, scale=None):
        y = _dot(src[pl.ds(_al(r, n), n), :], pltpu.bitcast(w[h], BF))
        dst[pl.ds(_al(r, n), n), :] = (y if scale is None else y * scale).astype(BF)

    def relayout_group(raw, g, dst, rows):
        _loop(0, rows // (16 * RLU),
              lambda i: [_relayout16(raw, g, (i * RLU + u) * 16, dst) for u in range(RLU)])

    for q in (c_c, c_wm0):
        q.start()
    _loop(0, NX, lambda i: x_copy(i).start())
    c_wq[0].start()
    c_c.wait()
    c_wm0.wait()
    c_wk[0].start()
    c_wv[0].start()
    cc = c_v[...].astype(F32)
    sc = (cc * jax.nn.sigmoid(cc)).astype(BF)
    mod_s[:, 0:2 * M] = _dot(sc, wmod_v[:, 0:2 * M])
    sa = mod_s[:, 0:M]
    ca = mod_s[:, M:2 * M]

    def ln_chunk(i):
        x_copy(i).wait()
        r = _al(i * xr, xr)
        xx = x_v[pl.ds(r, xr), :].astype(F32)
        h1_s[pl.ds(r, xr), :] = (_ln(xx) * (1.0 + ca) + sa).astype(BF)
    _loop(0, NX, ln_chunk)

    c_wq[0].wait()
    _loop(0, NX, lambda i: ck_copy(i).start())
    relayout_group(wq_v, 0, wq2, M)
    _loop(0, NX, lambda i: project(h1_s, wq2, 0, qa, i * xr, xr, QSCALE))
    c_wk[0].wait()
    relayout_group(wk_v, 0, wk2, DC)
    c_wv[0].wait()
    for q in (c_wk[1], c_wv[1], c_wq[1]):
        q.start()
    relayout_group(wv_v, 0, wv2, DC)

    def kv_chunk(i):
        ck_copy(i).wait()
        project(ckv_v, wk2, 0, ka, i * xr, xr)
        project(ckv_v, wv2, 0, va, i * xr, xr)
    _loop(0, NX, kv_chunk)

    tri = lax.broadcasted_iota(jnp.int32, (BQ, BQ), 1) <= lax.broadcasted_iota(jnp.int32, (BQ, BQ), 0)

    def proj_pieces(h, qd, kd, vd):
        pcs = []
        for r in range(S // PC):
            pcs.append(lambda r=r: project(ckv_v, wk2, h, kd, r * PC, PC))
            pcs.append(lambda r=r: project(ckv_v, wv2, h, vd, r * PC, PC))
            pcs.append(lambda r=r: project(h1_s, wq2, h, qd, r * PC, PC, QSCALE))
        return pcs

    def qk(i, qs, ks):
        q0 = i * BQ
        s = _dot_nt(qs[q0:q0 + BQ, :], ks[0:q0 + BQ, :])
        sd = jnp.where(tri, s[:, q0:], NEG)
        return jnp.concatenate([s[:, :q0], sd], axis=1) if i > 0 else sd

    def softmax(s):
        m = jnp.max(s, axis=1, keepdims=True)
        p = jnp.exp2(s - m)
        return p.astype(BF), jnp.sum(p, axis=1, keepdims=True)

    def pv(i, hd, p, l, vs):
        q0 = i * BQ
        o = _dot(p, vs[0:q0 + BQ, :]) * (1.0 / l)
        ctx_s[hd, q0:q0 + BQ, :] = o.astype(BF)

    order = list(range(NS))[0::2] + list(range(NS))[1::2][::-1]

    def share(nf):
        return [(nf * (n + 1)) // NS - (nf * n) // NS for n in range(NS)]

    def head_pair(ha, hb, fa, fb):
        tasks = [(ha, i, qa, ka, va) for i in order] + [(hb, i, qb, kb, vb) for i in order]
        nt = len(tasks)
        quota = share(len(fa)) + share(len(fb))
        scores = {0: qk(*tasks[0][1:4])}
        probs = {}

        def do_q(n):
            if n + 1 < nt:
                scores[n + 1] = qk(*tasks[n + 1][1:4])

        def do_p(n):
            if 0 <= n - 1 < nt:
                hd, i, _, _, vs = tasks[n - 1]
                pv(i, hd, *probs.pop(n - 1), vs)

        for n in range(nt + 1):
            fill = fa if n < NS else fb
            if n < NS or fb:
                do_p(n)
                for _ in range(quota[n] if n < nt else 0):
                    fill.pop(0)()
                do_q(n)
            else:
                do_q(n)
                do_p(n)
            if n < nt:
                probs[n] = softmax(scores.pop(n))

    def pair_body(p):
        @pl.when(p == 1)
        def _():
            for q in (c_wk[1], c_wv[1], c_wq[1]):
                q.wait()
            for q in (c_wm1, c_wo, c_w1, c_w2, c_w3, c_w4):
                q.start()
            relayout_group(wk_v, 1, wk2, DC)
            relayout_group(wv_v, 1, wv2, DC)
            relayout_group(wq_v, 1, wq2, M)
        head_pair(2 * p, 2 * p + 1, proj_pieces(2 * p + 1, qb, kb, vb), proj_pieces(2 * p + 2, qa, ka, va))
    _loop(0, H // 2 - 1, pair_body)

    c_wm1.wait()
    mod_s[:, 2 * M:6 * M] = _dot(sc, wmod_v[:, 2 * M:6 * M])
    c_wo.wait()
    c_w1.wait()
    zpad = jnp.zeros((8, M), F32)
    t_s[0:8, :] = zpad
    t_s[S + 8:S + 16, :] = zpad
    head_pair(H - 2, H - 1, proj_pieces(H - 1, qb, kb, vb), [])

    def modp(j):
        return mod_s[:, j * M:(j + 1) * M]

    def out_proj(r, n):
        acc = jnp.zeros((n, M), F32)
        for hd in range(H):
            acc += _dot(ctx_s[hd, pl.ds(_al(r, 16), n), :], wo_v[hd * D:(hd + 1) * D, :])
        xa = x_v[pl.ds(_al(r, 16), n), :].astype(F32) + modp(2) * acc
        xa_s[pl.ds(_al(r, 8), n), :] = xa
        return xa

    def ada_ln(r, n, xa):
        hb = _ln(xa) * (1.0 + modp(4)) + modp(3)
        hb_s[pl.ds(_al(r, 8), n), :] = hb
        return _ln(hb).astype(BF)

    def mlp1(i):
        r, n = i * RB, RB // SUB1
        xs, hl = [None] * n, [None] * n
        for k in range(n + 2):
            if k < n:
                xs[k] = out_proj(r + k * SUB1, SUB1)
            if 0 <= k - 2 < n:
                t_s[pl.ds(_al(r + (k - 2) * SUB1 + 8, 8), SUB1), :] = _gelu(_dot(hl[k - 2], w1_v[...]))
            if 0 <= k - 1 < n:
                hl[k - 1] = ada_ln(r + (k - 1) * SUB1, SUB1, xs[k - 1])
    _loop(0, S // RB, mlp1)

    c_w2.wait()
    c_w3.wait()
    c_w4.wait()
    G = M // 4
    offs = (-1, 1, -2, 2)

    def shift_proj(r, n):
        lane = lax.broadcasted_iota(jnp.int32, (n, 128), 1)
        cols = []
        for ct in range(M // 128):
            g_lo, g_hi = (ct * 128) // G, (ct * 128 + 127) // G
            w = t_s[pl.ds(_al(r, 8), n + 16), ct * 128:(ct + 1) * 128]
            a = w[8 + offs[g_lo]:8 + offs[g_lo] + n]
            if g_hi != g_lo:
                a = jnp.where(lane < (g_hi * G - ct * 128), a, w[8 + offs[g_hi]:8 + offs[g_hi] + n])
            cols.append(a)
        g = jnp.concatenate(cols, axis=1).astype(BF)
        return hb_s[pl.ds(_al(r, 8), n), :] + _dot(g, w2_v[...])

    def finish(r, n, y1, u):
        y2 = y1 + _dot(u, w4_v[...])
        rows = pl.ds(_al(r, 16), n)
        ostage[rows, :] = (xa_s[pl.ds(_al(r, 8), n), :] + modp(5) * y2).astype(BF)
        pltpu.make_async_copy(ostage.at[rows, :], out_hbm.at[rows, :], osem.at[0]).start()

    def mlp2(i):
        r, n = i * RB, RB // SUB2
        y, l, u = [None] * n, [None] * n, [None] * n
        for k in range(n + 3):
            if k < n:
                y[k] = shift_proj(r + k * SUB2, SUB2)
            if 0 <= k - 3 < n:
                finish(r + (k - 3) * SUB2, SUB2, y[k - 3], u[k - 3])
            if 0 <= k - 2 < n:
                u[k - 2] = _gelu(_dot_nt(l[k - 2], w3_v[...])).astype(BF)
            if 0 <= k - 1 < n:
                l[k - 1] = _ln(y[k - 1]).astype(BF)
    _loop(0, S // RB, mlp2)
    pltpu.make_async_copy(ostage, out_hbm, osem.at[0]).wait()


@jax.jit
def pallas_adaLN_cond__compressed_kv_cla__mixer_s_mlp__prompt_kernel(
    A_x, A_c_kv, A_w_q, A_w_uk, A_w_uv, A_w_o, B_x, B_w1, B_w2, B_w3, B_w4, c, w_mod
):
    del B_x
    vmem = pltpu.VMEM
    scratch = [
        vmem((S, DC), BF), vmem((S, M), BF),
        vmem((H, M // 2, D), U32), vmem((H, DC // 2, D), U32), vmem((H, DC // 2, D), U32),
        vmem((H + 6, S, D), BF),
        vmem((H * D, M), BF), vmem((S, M), BF),
        vmem((S, M), F32), vmem((S, M), F32), vmem((S + 16, M), F32),
        vmem((M, M), BF), vmem((M, M), BF), vmem((F, M), BF), vmem((F, M), BF),
        vmem((S, M), BF), vmem((1, 6 * M), F32),
        vmem((2, M, GH, D), BF), vmem((2, DC, GH, D), BF), vmem((2, DC, GH, D), BF),
        vmem((1, M), BF), vmem((M, 6 * M), BF),
        pltpu.SemaphoreType.DMA((14,)), pltpu.SemaphoreType.DMA((NX,)), pltpu.SemaphoreType.DMA((NX,)),
        pltpu.SemaphoreType.DMA((1,)),
    ]
    hbm = pl.BlockSpec(memory_space=pltpu.HBM)
    out = pl.pallas_call(
        _kernel,
        out_shape=jax.ShapeDtypeStruct((S, M), BF),
        in_specs=[hbm] * 12,
        out_specs=hbm,
        scratch_shapes=scratch,
        compiler_params=pltpu.CompilerParams(vmem_limit_bytes=110 * 1024 * 1024),
    )(A_x.reshape(S, M), A_c_kv.reshape(S, DC), A_w_q, A_w_uk, A_w_uv, A_w_o.reshape(H * D, M),
      B_w1, B_w2, B_w3.T, B_w4, c, w_mod)
    return out.reshape(1, S, M)
```
